```python
import jax
import jax.numpy as jnp

def _softmax(x, axis=-1):
    return jax.nn.softmax(x, axis=axis)
def _gelu(x):
    return jax.nn.gelu(x, approximate=True)
def _silu(x):
    return jax.nn.silu(x)
def _sigmoid(x):
    return jax.nn.sigmoid(x)
def _layernorm(x, axis=-1, eps=1e-5):
    m = jnp.mean(x, axis=axis, keepdims=True)
    v = jnp.var(x, axis=axis, keepdims=True)
    return (x - m) / jnp.sqrt(v + eps)
def _scatter_add(tgt, idx, src, axis=0):
    return tgt.at[idx].add(src)
def _segment_sum(src, seg, n):
    return jax.ops.segment_sum(src, seg, n)
class _Rng:
    def __init__(self, key):
        self._k = key
    def _next(self):
        self._k, sub = jax.random.split(self._k)
        return sub
    def normal(self, shape):
        return jax.random.normal(self._next(), shape, dtype=jnp.bfloat16)
    def randint(self, lo, hi, shape):
        return jax.random.randint(self._next(), shape, lo, hi, dtype=jnp.int32)
    def uniform(self, shape, lo=0.0, hi=1.0):
        return jax.random.uniform(self._next(), shape, jnp.bfloat16, lo, hi)
    def permutation(self, n):
        return jax.random.permutation(self._next(), n)


kernel_name = 'interleave_layers__sliding_local_dilated__glu_gated_glu__prompt'

def setup_inputs():
    _rng = _Rng(jax.random.key(int.from_bytes(__import__("os").urandom(4), "little")))
    _w = (lambda a: (lambda t: t.astype(jnp.bfloat16) if jnp.issubdtype(t.dtype, jnp.floating) else t)(jnp.asarray(a)))
    def _A_setup():
        B, S, D = 1, 2048, 576
        return {
            "x": _w((lambda *s: _rng.normal(s) * 0.05)(B, S, D)),
            "wqkv": _w((lambda *s: _rng.normal(s) * 0.05)(D, 3 * D)),
            "wo": _w((lambda *s: _rng.normal(s) * 0.05)(D, D)),
        }
    _A_in = _A_setup()

    def _B_setup():
        B, S, D, F = 1, 2048, 576, 4608
        return {
            "x": _w((lambda *s: _rng.normal(s) * 0.05)(B, S, D)),
            "w_gate": _w((lambda *s: _rng.normal(s) * 0.05)(D, F)),
            "w_up": _w((lambda *s: _rng.normal(s) * 0.05)(D, F)),
            "w_down": _w((lambda *s: _rng.normal(s) * 0.05)(F, D)),
        }
    _B_in = _B_setup()

    return {
        "A_x": _A_in["x"],
        "A_wqkv": _A_in["wqkv"],
        "A_wo": _A_in["wo"],
        "B_x": _B_in["x"],
        "B_w_gate": _B_in["w_gate"],
        "B_w_up": _B_in["w_up"],
        "B_w_down": _B_in["w_down"],
    }

def reference(A_x, A_wqkv, A_wo, B_x, B_w_gate, B_w_up, B_w_down):
    def _A_ref(x, wqkv, wo):
        B, S, D = x.shape
        H = 32; Dh = D // H
        W, dil = 8, 2
        qkv = (lambda x, *d: x.transpose(*d))((x @ wqkv).reshape(B, S, 3, H, Dh), 2, 0, 3, 1, 4)
        q, k, v = qkv[0], qkv[1], qkv[2]
        scale = Dh ** -0.5
        pos = jnp.arange(S)
        off = jnp.arange(W) * dil
        idx = pos[:, None] - off[None, :]
        mask = idx >= 0
        idx_c = jnp.where(mask, idx, 0).reshape(-1)
        kg = k[:, :, idx_c, :].reshape(B, H, S, W, Dh)
        vg = v[:, :, idx_c, :].reshape(B, H, S, W, Dh)
        logits = jnp.einsum("bhsd,bhswd->bhsw", q, kg) * scale
        logits = jnp.where(mask[None, None, :, :], logits, -1e9)
        attn = _softmax(logits, axis=-1)
        o = jnp.einsum("bhsw,bhswd->bhsd", attn, vg)
        return (lambda x, *d: x.transpose(*d))(o, 0, 2, 1, 3).reshape(B, S, D) @ wo

    def _B_ref(x, w_gate, w_up, w_down):
        g = jnp.einsum("bsd,df->bsf", x, w_gate)
        u = jnp.einsum("bsd,df->bsf", x, w_up)
        h = _sigmoid(g) * u
        return jnp.einsum("bsf,fd->bsd", h, w_down)

    x = A_x
    x = x + _A_ref(_layernorm(x, axis=-1), A_wqkv, A_wo)
    x = x + _B_ref(_layernorm(x, axis=-1), B_w_gate, B_w_up, B_w_down)
    x = x + _A_ref(_layernorm(x, axis=-1), A_wqkv, A_wo)
    x = x + _B_ref(_layernorm(x, axis=-1), B_w_gate, B_w_up, B_w_down)
    return x
```

```python
import jax
import jax.numpy as jnp
from jax import lax
import jax.experimental.pallas as pl
import jax.experimental.pallas.tpu as pltpu

S, D, F = 2048, 576, 4608
NH, DH = 32, 18
WIN, DIL = 8, 2
NP = S // 256
HD = D // 2
KT = F // 256
R_GU = 128
R_SM = 96
R_DN = 96

f32, bf16, u32 = jnp.float32, jnp.bfloat16, jnp.uint32


def _pack(x):
    return pltpu.bitcast(x.astype(bf16), u32)


def _dot(w_words, x_words):
    return jnp.dot(pltpu.bitcast(w_words, bf16), pltpu.bitcast(x_words, bf16),
                   preferred_element_type=f32)


def _even_rows(words):
    return pltpu.bitcast(words << 16, f32)


def _odd_rows(words):
    return pltpu.bitcast(words & jnp.uint32(0xFFFF0000), f32)


def _w_operands(w1, w2):
    lo = lax.broadcasted_iota(jnp.int32, w1[0].shape, 1) < 64
    e6, e7 = w2[2] - w1[2], w1[3] - w2[3]
    return [
        w1[0] + w2[1], w2[0] + w2[1], w1[0], w2[1], w1[0] + w1[1],
        w2[0] - w1[0], w1[1] - w2[1],
        w1[2] + w2[3], w2[2] + w2[3],
        jnp.where(lo, w1[2], w2[3]), jnp.where(lo, w2[3], w1[2]),
        w1[2] + w1[3],
        jnp.where(lo, e6, w2[4]), jnp.where(lo, e7, w1[4]),
        jnp.where(lo, w2[4], e6), jnp.where(lo, w1[4], e7),
    ]


def _x_operands(get, dst, n=32):
    def put(i, r, v):
        dst[i, r // 2:(r + n) // 2, :] = _pack(v)

    for r in range(0, 192, n):
        first = r < 128
        x11, x12 = get(r if first else r + 128, n)
        x21, x22 = get(r + 128 if first else r + 256, n)
        ops = [x11 + x22, x11, x12 - x22, x21 - x11, x22, x11 + x12, x21 + x22]
        for i, v in enumerate(ops):
            put(i if first else i + 7, r % 128, v)
    for r in range(64, 128, n):
        x11, x12 = get(256 + r, n)
        x21, x22 = get(384 + r, n)
        put(16, r, x12 + x21)
        put(8, r, -x12)
        put(9, r, x22 - x12)
        put(10, r, x11 - x21)
        put(11, r, -x21)
        put(14, r, x11 + x12)
        put(15, r, x21 + x22)
    for r in range(0, 64, n):
        s1, s2 = get(512 + r, n)
        put(12, 64 + r, s2)
        put(13, 64 + r, s1)
        put(14, r, s1)
        put(15, r, s2)


def _mm17(w_ref, r0, rows, x_ref):
    def p(i, j=None):
        return _dot(w_ref[i, r0 // 2:(r0 + rows) // 2, :],
                    x_ref[i if j is None else j])

    g1 = p(0) + p(7)
    g4 = p(3) + p(10)
    g5 = p(4) + p(11)
    c11 = (g1 + g4) - g5 + p(6) + p(13)
    g10 = p(7, 16)
    g3 = p(2) + p(9)
    c12 = (g5 + g10) + g3 + p(15)
    g2 = p(1) + p(8)
    c21 = (g4 + g10) + g2 + p(14)
    c22 = (g1 + g3) - g2 + p(5) + p(12)
    return c11, c12, c21, c22


def _layernorm_operands(res, p, dst, scale):
    stats = []
    for t in (2 * p, 2 * p + 1):
        mean = jnp.sum(res[t], axis=0, keepdims=True) * (1.0 / D)
        c = res[t] - mean
        var = jnp.sum(c * c, axis=0, keepdims=True) * (1.0 / D)
        stats.append((t, mean, lax.rsqrt(var + 1e-5) * scale))

    def get(r, n):
        return [(res[t, r:r + n, :] - m) * rs for t, m, rs in stats]

    _x_operands(get, dst)


def _attention(qs, ks, vs, p, os_):
    lane = lax.broadcasted_iota(jnp.int32, (8, 128), 1)
    n_masked = jnp.where(p == 0, DIL, 0)

    def window(ref, r):
        t = [ref[2 * p + i, r:r + 8, :] for i in range(3)]
        out = []
        for i in range(2):
            sh = [t[i + 1]]
            for w in range(1, WIN):
                s = DIL * w
                sh.append(pltpu.roll(jnp.where(lane >= 128 - s, t[i], t[i + 1]), s, 1))
            out.append(sh)
        return out

    for h0 in range(0, NH, 8):
        acc = [[None] * WIN for _ in range(2)]
        for d in range(DH):
            r = d * NH + h0
            kw = window(ks, r)
            for i in range(2):
                q = qs[2 * p + i, r:r + 8, :]
                for w in range(WIN):
                    t = q * kw[i][w]
                    acc[i][w] = t if d == 0 else acc[i][w] + t
        prob = []
        for i in range(2):
            lg = [a * (DH ** -0.5) for a in acc[i]]
            if i == 0:
                lg = [lg[0]] + [jnp.where(lane < n_masked * w, -1e9, lg[w])
                                for w in range(1, WIN)]
            m = lg[0]
            for w in range(1, WIN):
                m = jnp.maximum(m, lg[w])
            e = [jnp.exp(v - m) for v in lg]
            tot = e[0]
            for w in range(1, WIN):
                tot = tot + e[w]
            inv = 1.0 / tot
            prob.append([v * inv for v in e])
        for d in range(DH):
            r = d * NH + h0
            vw = window(vs, r)
            for i in range(2):
                o = prob[i][0] * vw[i][0]
                for w in range(1, WIN):
                    o = o + prob[i][w] * vw[i][w]
                os_[i, r:r + 8, :] = o


def _k_tiles(raw, c0, c1):
    tiles = [raw[128 * t:128 * (t + 1), c0:c1] for t in range(4)]
    tail = raw[512:D, c0:c1]
    return tiles + [jnp.concatenate([tail, tail], axis=0)]


def _kernel(x_hbm, wqkv_hbm, wo_hbm, wg_hbm, wu_hbm, wd_hbm, out_hbm,
            xin, wqkv_raw, wo_raw, wg_raw, wu_raw, wd_raw, obuf,
            tmp, wq_s, wo_s, wgu_s, wd_s,
            res, qs, ks, vs, os_, xq, xo, xg, hs, sem_in, sem_out):
    cp_qkv = pltpu.make_async_copy(wqkv_hbm, wqkv_raw, sem_in.at[0])
    cp_x = [pltpu.make_async_copy(x_hbm.at[:, 256 * p:256 * (p + 1)], xin.at[p],
                                  sem_in.at[5 + p]) for p in range(NP)]
    cp_wo = pltpu.make_async_copy(wo_hbm, wo_raw, sem_in.at[1])
    cp_wg = pltpu.make_async_copy(wg_hbm, wg_raw, sem_in.at[2])
    cp_wu = pltpu.make_async_copy(wu_hbm, wu_raw, sem_in.at[3])
    cp_wd = pltpu.make_async_copy(wd_hbm, wd_raw, sem_in.at[4])
    for cp in [cp_qkv] + cp_x + [cp_wo]:
        cp.start()

    def out_copy(p):
        col = pl.ds(pl.multiple_of(p * 256, 256), 256)
        return pltpu.make_async_copy(obuf.at[p], out_hbm.at[:, col], sem_out.at[p])

    for ref in (xq, xo, xg):
        ref[7, 32:64, :] = jnp.zeros((32, 128), u32)
        ref[16, 0:32, :] = jnp.zeros((32, 128), u32)
    ks[0] = jnp.zeros((D, 128), f32)

    def prep_wqkv():
        for t, tile in enumerate(_k_tiles(wqkv_raw, 0, 3 * D)):
            tmp[t] = pltpu.bitcast(tile.T, u32)
        for m in range(3):
            for j in range(DH // 2):
                words = [tmp[t, pl.ds(m * HD + j, NH, stride=DH // 2), :]
                         for t in range(5)]
                ops = _w_operands([_even_rows(v) for v in words],
                                  [_odd_rows(v) for v in words])
                r = (m * HD + j * NH) // 2
                for i, v in enumerate(ops):
                    wq_s[i, r:r + NH // 2, :] = _pack(v)

    def prep_wo():
        for c in range(4):
            tmp[c, 0:HD, :] = pltpu.bitcast(wo_raw[:, 128 * c:128 * (c + 1)], u32)
        tmp[4, 0:HD, 0:64] = pltpu.bitcast(wo_raw[:, 512:D], u32)
        wt = []
        for t in range(5):
            dd = [4 * t + i for i in range(4)] if t < 4 else [16, 17, 16, 17]
            cols = []
            for c in range(5):
                rows = []
                for d in dd:
                    words = tmp[c, pl.ds(d % 9, NH, stride=DH // 2), :]
                    rows.append(_even_rows(words) if d < 9 else _odd_rows(words))
                cols.append(jnp.concatenate(rows, axis=0).T)
            wt.append(jnp.concatenate(cols, axis=0))
        for r in range(0, HD, 32):
            ops = _w_operands([v[r:r + 32] for v in wt],
                              [v[HD + r:HD + r + 32] for v in wt])
            for i, v in enumerate(ops):
                wo_s[i, r // 2:r // 2 + 16, :] = _pack(v)

    def prep_gate_up(b):
        half = R_GU // 2
        for m, raw in enumerate((wg_raw, wu_raw)):
            wt = [tile.T for tile in _k_tiles(raw, 256 * b, 256 * (b + 1))]
            for r in range(0, 128, 32):
                ops = _w_operands([v[r:r + 32].astype(f32) for v in wt],
                                  [v[128 + r:160 + r].astype(f32) for v in wt])
                row = 256 * b + (r // half) * R_GU + m * half + r % half
                for i, v in enumerate(ops):
                    wgu_s[i, row // 2:row // 2 + 16, :] = _pack(v)

    def prep_down(b):
        for r in range(0, HD, 32):
            w11, w12, w21, w22 = [
                wd_raw[r0 + r:r0 + r + 32, c0:c0 + 128].astype(f32)
                for r0 in (0, HD) for c0 in (256 * b, 256 * b + 128)]
            ops = [w11 + w22, w21 + w22, w11, w22, w11 + w12, w21 - w11, w12 - w22]
            for i, v in enumerate(ops):
                wd_s[i * KT + b, r // 2:r // 2 + 16, :] = _pack(v)

    def load_x(p):
        for i in range(2):
            res[2 * p + i] = xin[p, :, 128 * i:128 * (i + 1)].astype(f32)

    def qkv(p):
        for m, (dst, off) in enumerate(((qs, 0), (ks, 1), (vs, 1))):
            for r in range(0, HD, R_SM):
                c = _mm17(wq_s, m * HD + r, R_SM, xq)
                for n, v in enumerate(c):
                    r0 = (n // 2) * HD + r
                    dst[2 * p + n % 2 + off, r0:r0 + R_SM, :] = v

    def first_token_halo():
        vs[0] = jnp.broadcast_to(vs[1, :, 0:1], (D, 128))

    def attend(p):
        _attention(qs, ks, vs, p, os_)
        _x_operands(lambda r, n: (os_[0, r:r + n, :], os_[1, r:r + n, :]), xo)

    def project(p):
        for r in range(0, HD, R_SM):
            c = _mm17(wo_s, r, R_SM, xo)
            for n, v in enumerate(c):
                r0 = (n // 2) * HD + r
                res[2 * p + n % 2, r0:r0 + R_SM, :] += v
        _layernorm_operands(res, p, xg, 0.5)

    def gate_up(b):
        half = R_GU // 2
        for r in range(256 * b, 256 * (b + 1), R_GU):
            h11, h12, h21, h22 = [
                jnp.tanh(c[:half]) * c[half:] + c[half:]
                for c in _mm17(wgu_s, r, R_GU, xg)]
            ops = [h11 + h22, h11, h12 - h22, h21 - h11, h22, h11 + h12, h21 + h22]
            for i, v in enumerate(ops):
                hs[i, r // 4:(r + R_GU) // 4, :] = _pack(v)

    def down(p):
        for r in range(0, HD, R_DN):
            def prod(i):
                acc = None
                for k in range(KT):
                    t = _dot(wd_s[i * KT + k, r // 2:(r + R_DN) // 2, :],
                             hs[i, 64 * k:64 * (k + 1), :])
                    acc = t if acc is None else acc + t
                return acc

            def emit(n, v):
                r0 = (n // 2) * HD + r
                v = v + res[2 * p + n % 2, r0:r0 + R_DN, :]
                res[2 * p + n % 2, r0:r0 + R_DN, :] = v
                obuf[p, r0:r0 + R_DN, 128 * (n % 2):128 * (n % 2 + 1)] = v.astype(bf16)

            m1, m4, m5 = prod(0), prod(3), prod(4)
            emit(0, (m1 + m4) - m5 + prod(6))
            m3 = prod(2)
            emit(1, m3 + m5)
            m2 = prod(1)
            emit(2, m2 + m4)
            emit(3, (m1 + m3) - m2 + prod(5))

    cp_qkv.wait()
    for cp in (cp_wg, cp_wu, cp_wd):
        cp.start()
    prep_wqkv()
    for cp in cp_x:
        cp.wait()
    cp_wo.wait()
    load_x(0)
    _layernorm_operands(res, 0, xq, 1.0)

    def qkv_step(p, carry):
        qkv(p)
        load_x(p + 1)
        _layernorm_operands(res, p + 1, xq, 1.0)
        return carry

    lax.fori_loop(0, NP - 1, qkv_step, 0)
    first_token_halo()
    attend(0)
    prep_wo()
    qkv(NP - 1)
    project(0)

    cp_wg.wait()
    cp_wu.wait()
    cp_wd.wait()
    prep_gate_up(0)
    attend(1)
    for b in range(KT):
        if b + 1 < KT:
            prep_gate_up(b + 1)
        gate_up(b)
        prep_down(b)
    project(1)
    down(0)

    def step(s, with_qkv):
        p, nxt, prv = s % NP, (s + 1) % NP, s - 1
        if with_qkv:
            pl.when(nxt == 0)(first_token_halo)
            _layernorm_operands(res, prv, xq, 1.0)
        attend(nxt)
        for b in range(KT):
            gate_up(b)
        project(nxt)
        if with_qkv:
            qkv(prv)
        down(p)

    def step_a(s, carry):
        step(s, True)
        return carry

    def step_b(s, carry):
        out_copy(s - NP - 1).start()
        step(s, False)
        return carry

    lax.fori_loop(1, NP + 1, step_a, 0)
    lax.fori_loop(NP + 1, 2 * NP, step_b, 0)
    out_copy(NP - 1).start()
    for p in range(NP):
        out_copy(p).wait()


@jax.jit
def pallas_interleave_layers__sliding_local_dilated__glu_gated_glu__prompt_kernel(
    A_x: jax.Array,
    A_wqkv: jax.Array,
    A_wo: jax.Array,
    B_x: jax.Array,
    B_w_gate: jax.Array,
    B_w_up: jax.Array,
    B_w_down: jax.Array,
):
    del B_x
    vmem = pltpu.VMEM
    out = pl.pallas_call(
        _kernel,
        out_shape=jax.ShapeDtypeStruct((D, S), bf16),
        in_specs=[pl.BlockSpec(memory_space=pl.ANY)] * 6,
        out_specs=pl.BlockSpec(memory_space=pl.ANY),
        scratch_shapes=[
            vmem((NP, D, 256), bf16),
            vmem((D, 3 * D), bf16),
            vmem((D, D), bf16),
            vmem((D, F), bf16),
            vmem((D, F), bf16),
            vmem((D, F), bf16),
            vmem((NP, D, 256), bf16),
            vmem((5, 3 * HD, 128), u32),
            vmem((16, 3 * HD // 2, 128), u32),
            vmem((16, HD // 2, 128), u32),
            vmem((16, F // 2, 128), u32),
            vmem((7 * KT, HD // 2, 128), u32),
            vmem((2 * NP, D, 128), f32),
            vmem((2 * NP, D, 128), f32),
            vmem((2 * NP + 1, D, 128), f32),
            vmem((2 * NP + 1, D, 128), f32),
            vmem((2, D, 128), f32),
            vmem((17, 64, 128), u32),
            vmem((17, 64, 128), u32),
            vmem((17, 64, 128), u32),
            vmem((7, F // 4, 128), u32),
            pltpu.SemaphoreType.DMA((5 + NP,)),
            pltpu.SemaphoreType.DMA((NP,)),
        ],
        compiler_params=pltpu.CompilerParams(vmem_limit_bytes=110 * 1024 * 1024),
        name="interleaved_attn_glu",
    )(A_x.reshape(S, D).T, A_wqkv, A_wo, B_w_gate, B_w_up, B_w_down.T)
    return out.T.reshape(1, S, D)
```

```python
import jax
import jax.numpy as jnp
from jax import lax
import jax.experimental.pallas as pl
import jax.experimental.pallas.tpu as pltpu

S, D, F = 2048, 576, 4608
NH, DH = 32, 18
WIN, DIL = 8, 2
NP = S // 256
K_GU, K_QKV, K_O = 4, 2, 2
M_DN = 6
R_GU = 64
LN_SUM, LN_SQ, LN_OUT = 64, 48, 48
Q0, K0, V0 = 0, 2 * NP + 1, 4 * NP + 2
FIRST = (0, 128, 256, 384, 448)

f32, bf16, u32 = jnp.float32, jnp.bfloat16, jnp.uint32


def _ds(start, n, align=8):
    return pl.ds(start if isinstance(start, int) else pl.multiple_of(start, align), n)


def _put(ref, i, r, v):
    n = v.shape[0]
    if v.dtype == bf16:
        ref.bitcast(u32)[i, r // 2:(r + n) // 2, :] = pltpu.bitcast(v, u32)
    else:
        ref[i, r:r + n, :] = v.astype(bf16)


def _get(ref, i, r, n):
    if n % 16:
        return ref[i, r:r + n, :]
    return pltpu.bitcast(ref.bitcast(u32)[i, r // 2:(r + n) // 2, :], bf16)


def _dot(w, x):
    return jnp.dot(w, x, preferred_element_type=f32)


def _even_rows(words):
    return pltpu.bitcast(words << 16, f32)


def _odd_rows(words):
    return pltpu.bitcast(words & jnp.uint32(0xFFFF0000), f32)


class _Background:
    def __init__(self, zero):
        self.zero, self.jobs = zero, []

    def add(self, pieces, rate=1.0, delay=0):
        self.jobs.append([pieces, rate, -rate * delay, next(pieces)])

    def _advance(self, job):
        job[3] = next(job[0], None)

    def tick(self, v):
        for job in self.jobs:
            job[2] += job[1]
            fenced = None
            while job[2] >= 1 and job[3] is not None:
                ref = job[3]
                if ref is not fenced:
                    n = 32 // ref.dtype.itemsize
                    val = pltpu.bitcast(v[:n], u32) if ref.dtype == u32 else v[:n].astype(ref.dtype)
                    ref[self.zero, ref.shape[1] - n:, 0:128] = val
                    fenced = ref
                job[2] -= 1
                self._advance(job)

    def finish(self):
        for job in self.jobs:
            while job[3] is not None:
                self._advance(job)
        self.jobs = []


def _plan(m, row_a, row_b):
    plan = []
    for i in range(m):
        a, al = row_a(i), i
        others = [j for j in range(m) if j != i]
        plan.append([
            ([(1, a, al)] + [(1, a, m + j) for j in others],
             [(1, al, 1)], [(-1, a, 0), (1, a, 1)]),
            ([(1, a, al)] + [(-1, row_b(j), al) for j in others],
             [(1, al, 0), (1, al, 1)], [(1, a, 0)])])
        for j in others:
            b, be = row_b(j), m + j
            plan.append([
                ([(1, a, be), (1, b, al)], [(1, be, 0), (1, al, 1)], [(1, a, 0), (1, b, 1)]),
                ([(1, a, be)], [(1, be, 1), (-1, al, 1)], [(1, a, 1), (1, b, 1)]),
                ([(1, b, al)], [(1, al, 0), (-1, be, 0)], [(1, a, 0), (1, b, 0)])])
            if i == (m - 1 if j < m - 1 else m - 2):
                mates = [n for n in range(m) if n != j]
                plan.append([
                    ([(1, b, be)] + [(1, b, n) for n in mates],
                     [(1, be, 0)], [(1, b, 0), (-1, b, 1)]),
                    ([(1, b, be)] + [(-1, row_a(n), be) for n in mates],
                     [(1, be, 0), (1, be, 1)], [(1, b, 1)])])
    return plan


def _plan576(k):
    return _plan(k, lambda i: i, lambda i: k + i)


def _signed_sum(terms, value):
    acc = value(*terms[0][1:])
    for s, *key in terms[1:]:
        acc = acc + value(*key) if s > 0 else acc - value(*key)
    return acc


def _run(plan, product, emit, reps, tick, before=None):
    last = {}
    for n, batch in enumerate(plan):
        for _, _, outs in batch:
            for _, r, t in outs:
                last[r, t] = n
    acc = {}

    def add(s, r, t, v):
        if (r, t) in acc:
            acc[r, t] = acc[r, t] + v if s > 0 else acc[r, t] - v
        else:
            acc[r, t] = v

    base = 0
    for n, batch in enumerate(plan):
        if before is not None:
            before(batch, add)
        vals = [None] * len(batch)
        for rep in range(reps):
            for i, prod in enumerate(batch):
                v = product((base + i) * reps + rep, prod, rep)
                vals[i] = v if rep == 0 else vals[i] + v
            tick(v)
        terms = [(s, r, t, v) for (_, _, outs), v in zip(batch, vals) for s, r, t in outs]
        for term in sorted(terms, key=lambda t: -t[0]):
            add(*term)
        for key in sorted(acc):
            if last[key] == n:
                emit(*key, acc.pop(key))
        base += len(batch)


def _tile576(k, blk, rep):
    t = (blk % k) * (4 // k) + rep
    return 448 if (t == 3 and blk >= k) else 128 * t


def _count576(k):
    return sum(len(b) for b in _plan576(k)) * (4 // k)


def _classes(k, j):
    return (j, k + j) if j == k - 1 else (k + j, j)


def _share(k, j, w):
    r0, r1 = _classes(k, j)
    a, b = w(r1, 384), w(r0, 448)
    lo = lax.broadcasted_iota(jnp.int32, a.shape, 1) < 64
    return (jnp.where(lo, a, b), w(r0, 384) - jnp.where(lo, a, 0.0),
            w(r1, 448) - jnp.where(lo, 0.0, b))


def _w_operands(k, w, put):
    tiles = {(r, c): w(r, c) for r in range(2 * k) for c in FIRST}
    for j in range(k):
        r0, r1 = _classes(k, j)
        v, tiles[r0, 384], tiles[r1, 448] = _share(k, j, lambda *key: tiles[key])
        put(_count576(k) + j, v)
    n = 0
    for batch in _plan576(k):
        for terms, _, _ in batch:
            for rep in range(4 // k):
                put(n, _signed_sum(terms, lambda r, b: tiles[r, _tile576(k, b, rep)]))
                n += 1


def _slots(k):
    slot, n = {}, 0
    for batch in _plan576(k):
        for terms, _, _ in batch:
            for rep in range(4 // k):
                if len(terms) == 1 or len(batch) == 2:
                    slot.setdefault((terms[0][1], _tile576(k, terms[0][2], rep)), n)
                n += 1
    for j in range(k):
        r0, r1 = _classes(k, j)
        slot[r1, 384], slot[r0, 448] = n + j, n + k + j
    return slot


def _x_operands(k, ref, t0):
    x = {c: [ref[t0 + t, c:c + 128, :] for t in range(2)] for c in FIRST}
    ops = []
    for batch in _plan576(k):
        for _, terms, _ in batch:
            for rep in range(4 // k):
                ops.append(_signed_sum(terms, lambda b, t: x[_tile576(k, b, rep)][t]))
    for t in range(2):
        ops.append(jnp.concatenate([x[384][t][:64], x[448][t][64:]], axis=0))
    return [v.astype(bf16) for v in ops]


def _mm576(k, w, x, emit, tick):
    done = set()

    def shared(batch, add):
        j = batch[0][2][0][1] % k
        if j not in done:
            done.add(j)
            n = _count576(k)
            for t in range(2):
                v = _dot(w(n + j), x[n + t])
                add(1, j, t, v)
                add(1, k + j, t, v)

    _run(_plan576(k), lambda n, prod, rep: _dot(w(n), x[n]), emit, 4 // k, tick, shared)


def _row_groups(total, target):
    units = total // 16
    n = max(1, total // target)
    sizes = [16 * (units // n + (i < units % n)) for i in range(n)]
    sizes[-1] += total % 16
    return [(sum(sizes[:i]), sizes[i]) for i in range(n)]


def _layernorm(src, p, dst, scale):
    def column_mean(term, rows):
        acc = None
        for r in range(0, D, 8):
            if r % rows == 0:
                yield src
            acc = term(r) if r == 0 else acc + term(r)
        return jnp.broadcast_to(jnp.sum(acc * (1.0 / D), axis=0, keepdims=True), (8, 128))

    for t in range(2):
        def x(r):
            return src[2 * p + t, r:r + 8, :]

        def sq(r):
            c = x(r) - mean
            return c * c

        mean = yield from column_mean(x, LN_SUM)
        var = yield from column_mean(sq, LN_SQ)
        rs = lax.rsqrt(var + 1e-5) * scale
        for r in range(0, D, 8):
            if r % LN_OUT == 0:
                yield src
            dst[t, r:r + 8, :] = (x(r) - mean) * rs


def _attention(buf, p, out, i, h0):
    lane = lax.broadcasted_iota(jnp.int32, (8, 128), 1)
    tile = 2 * p + i

    def rows(d):
        return _ds(d * NH + h0, 8)

    def window(t, d):
        prev, cur = buf[t - 1, rows(d), :], buf[t, rows(d), :]
        return [cur] + [
            pltpu.roll(jnp.where(lane >= 128 - s, prev, cur), s, 1)
            for s in range(DIL, DIL * WIN, DIL)]

    for d in range(DH):
        yield buf
        q = buf[Q0 + tile, rows(d), :]
        terms = [q * k for k in window(K0 + tile, d)]
        acc = terms if d == 0 else [a + t for a, t in zip(acc, terms)]
    n_masked = jnp.where(tile == 0, DIL, 0)
    lg = [a * (DH ** -0.5) for a in acc]
    lg[1:] = [jnp.where(lane < n_masked * w, -1e9, lg[w]) for w in range(1, WIN)]
    m = lg[0]
    for v in lg[1:]:
        m = jnp.maximum(m, v)
    e = [jnp.exp(v - m) for v in lg]
    tot = e[0]
    for v in e[1:]:
        tot = tot + v
    inv = 1.0 / tot
    prob = [v * inv for v in e]
    for _ in range(1):
        yield buf
    for d in range(DH):
        yield buf
        terms = [a * v for a, v in zip(prob, window(V0 + tile, d))]
        o = terms[0]
        for t in terms[1:]:
            o = o + t
        out[i, rows(d), :] = o


PLAN_DN = _plan(M_DN, lambda i: i, lambda i: i)
REP_DN = F // 128 // (2 * M_DN)
R_DN = D // M_DN
F_GU = K_GU * R_GU
GROUPS = F // F_GU
PARTS_GU = NP - 2
F_PART = F // PARTS_GU
G_PART = GROUPS // PARTS_GU
T_GU = _count576(K_GU) + 2 * K_GU


def _kernel(x_hbm, wqkv_hbm, wo_hbm, wg_hbm, wu_hbm, wd_hbm, out_hbm,
            xin, wqkv_raw, wo_raw, wgu_raw, wd_raw, obuf,
            tmp, wq_s, wo_s, wgu_s, wd_s,
            res, mid, att, n1, n2, ao, hs, zeros, sem_in, sem_out):
    qkv_cols = (slice(0, 640), slice(640, 1152), slice(1152, 3 * D))

    def qkv_copy(m):
        c = qkv_cols[m]
        return pltpu.make_async_copy(wqkv_hbm.at[:, c], wqkv_raw.at[0, 0:D, c], sem_in.at[m])

    wo_copy = pltpu.make_async_copy(wo_hbm, wo_raw.at[0, 0:D], sem_in.at[3])

    def x_copy(p):
        return pltpu.make_async_copy(
            x_hbm.at[:, _ds(256 * p, 256, 256)], xin.at[p, 0:D], sem_in.at[4 + p])

    def gu_copy(n, m):
        return pltpu.make_async_copy(
            (wg_hbm, wu_hbm)[m].at[:, _ds(F_PART * n, F_PART, 128)],
            wgu_raw.at[2 * n + m, 0:D], sem_in.at[4 + NP + 2 * n + m])

    def down_copy(rep):
        c = slice(F // REP_DN * rep, F // REP_DN * (rep + 1))
        return pltpu.make_async_copy(
            wd_hbm.at[:, c], wd_raw.at[0, 0:D, c], sem_in.at[4 + NP + 2 * PARTS_GU + rep])

    copies = [qkv_copy(0), x_copy(0), qkv_copy(1), qkv_copy(2), x_copy(1), x_copy(2), wo_copy]
    for n in range(PARTS_GU):
        copies += [x_copy(p) for p in range(n + 3, min(n + 4, NP))] + [gu_copy(n, 0), gu_copy(n, 1)]
    copies += [down_copy(rep) for rep in range(REP_DN)]
    for cp in copies:
        cp.start()

    def out_copy(p):
        col = pl.ds(pl.multiple_of(p * 256, 256), 256)
        return pltpu.make_async_copy(obuf.at[p], out_hbm.at[:, col], sem_out.at[p])

    def fill(i, carry):
        zeros[i] = 0
        return carry

    lax.fori_loop(0, 2, fill, 0)
    att[K0 - 1, 0:D] = jnp.zeros((D, 128), f32)

    nq = NH // K_QKV

    def prep_wqkv(m):
        c = qkv_cols[m]
        for t, c0 in enumerate(FIRST):
            yield wqkv_raw
            tmp[t, c.start // 2:c.stop // 2, :] = pltpu.bitcast(wqkv_raw[0, c0:c0 + 128, c].T, u32)
        for j in range(9):
            yield tmp

            def w(blk, c):
                start = m * (D // 2) + j + 9 * nq * (blk // 2)
                words = tmp[FIRST.index(c), pl.ds(start, nq, stride=9), :]
                return _odd_rows(words) if blk % 2 else _even_rows(words)

            _w_operands(K_QKV, w, lambda i, v: _put(wq_s, i, (9 * m + j) * nq, v))

    def prep_wo():
        for c in range(5):
            yield wo_raw
            n = min(128, D - 128 * c)
            tmp[c, 0:D // 2, 0:n] = pltpu.bitcast(wo_raw[0, 0:D, 128 * c:128 * c + n], u32)
        for t, first in enumerate(FIRST):
            for c in range(5):
                yield tmp
                rows = []
                for d in range(first // NH, first // NH + 4):
                    words = tmp[c, pl.ds(d % 9, NH, stride=9), :]
                    rows.append(_even_rows(words) if d < 9 else _odd_rows(words))
                n = min(128, D - 128 * c)
                mid[t, 128 * c:128 * c + n, :] = jnp.concatenate(rows, axis=0).T[:n]
        size = D // (2 * K_O)
        for r in range(0, size, 16):
            yield mid
            yield mid
            _w_operands(K_O, lambda blk, c: mid[FIRST.index(c), blk * size + r:blk * size + r + 16, :],
                        lambda i, v: _put(wo_s, i, r, v))

    slot = _slots(K_GU)

    def transpose_gate_up(part):
        half = R_GU // 2
        for g in range(G_PART):
            for m in range(2):
                for c in FIRST:
                    yield wgu_raw
                    wt = wgu_raw[2 * part + m, c:c + 128, F_GU * g:F_GU * (g + 1)].T
                    for blk in range(2 * K_GU):
                        _put(wgu_s, part * T_GU + slot[blk, c], g * R_GU + m * half,
                             wt[blk * half:(blk + 1) * half])

    def combine_gate_up(part):
        reps, t0 = 4 // K_GU, part * T_GU
        for g in range(G_PART):
            def w(blk, c):
                return _get(wgu_s, t0 + slot[blk, c], r, n).astype(f32)

            n = 32
            for j in range(K_GU):
                r0, r1 = _classes(K_GU, j)
                for r in range(g * R_GU, (g + 1) * R_GU, n):
                    yield wgu_s
                    for key, v in zip(((r1, 384), (r0, 384), (r1, 448)), _share(K_GU, j, w)):
                        _put(wgu_s, t0 + slot[key], r, v)
            base = 0
            for batch in _plan576(K_GU):
                n = 16 if len(batch) == 2 else R_GU
                for r in range(g * R_GU, (g + 1) * R_GU, n):
                    for rep in range(reps):
                        yield wgu_s
                        vals = [(i, _signed_sum(terms, lambda a, b: w(a, _tile576(K_GU, b, rep))))
                                for i, (terms, _, _) in enumerate(batch) if len(terms) > 1]
                        for i, v in vals:
                            _put(wgu_s, t0 + (base + i) * reps + rep, r, v)
                base += len(batch)

    def prep_down(rep):
        def w(blk, kb):
            c = 128 * (rep * 2 * M_DN + kb)
            return wd_raw[0, blk * R_DN + r:blk * R_DN + r + 16, c:c + 128]

        for r in range(0, R_DN, 16):
            base = 0
            for batch in PLAN_DN:
                yield wd_raw
                for i, (terms, _, _) in enumerate(batch):
                    v = (w(*terms[0][1:]) if len(terms) == 1 else
                         _signed_sum(terms, lambda *key: w(*key).astype(f32)))
                    _put(wd_s, (base + i) * REP_DN + rep, r, v)
                base += len(batch)

    def load_x(p):
        for t in range(2):
            for r in range(0, D, 96):
                yield xin
                res[2 * p + t, r:r + 96, :] = xin[p, r:r + 96, 128 * t:128 * (t + 1)].astype(f32)
        yield from _layernorm(res, p, n1, 1.0)

    def qkv(p, xq, bg, parts=(0, 1, 2)):
        for m in parts:
            for r, n in _row_groups(9 * nq, 72):
                def emit(blk, t, v):
                    for i in range(0, n, nq):
                        row = ((blk % 2) * 9 + (r + i) // nq) * NH + nq * (blk // 2)
                        att[(Q0, K0, V0)[m] + 2 * p + t, row:row + nq, :] = v[i:i + nq]

                _mm576(K_QKV, lambda i: _get(wq_s, i, 9 * nq * m + r, n), xq, emit, bg.tick)

    def first_token_halo():
        att[V0 - 1, 0:D] = jnp.broadcast_to(att[V0, 0:D, 0:1], (D, 128))

    def project(p, bg, z):
        xo = _x_operands(K_O, ao, z)
        size = D // (2 * K_O)
        for r, n in _row_groups(size, 72):
            def emit(blk, t, v):
                rows = slice(blk * size + r, blk * size + r + n)
                mid[2 * p + t, rows, :] = res[2 * p + t, rows, :] + v

            _mm576(K_O, lambda i: _get(wo_s, i, r, n), xo, emit, bg.tick)
        bg.add(_layernorm(mid, p, n2, 0.5))

    def gate_up(g, xg, bg):
        half = R_GU // 2

        def emit(blk, t, v):
            r = F_GU * g + blk * half
            hs[t, r:r + half, :] = jnp.tanh(v[:half]) * v[half:] + v[half:]

        _mm576(K_GU, lambda i: _get(wgu_s, g // G_PART * T_GU + i, g % G_PART * R_GU, R_GU), xg, emit, bg.tick)

    def down(p, bg):
        def product(n, prod, rep):
            def h(kb, t):
                r = 128 * (rep * 2 * M_DN + kb)
                return hs[t, r:r + 128, :]

            return _dot(_get(wd_s, n, 0, R_DN), _signed_sum(prod[1], h).astype(bf16))

        def emit(blk, t, v):
            r = blk * R_DN
            v = v + mid[2 * p + t, r:r + R_DN, :]
            res[2 * p + t, r:r + R_DN, :] = v
            obuf[p, r:r + R_DN, 128 * t:128 * (t + 1)] = v.astype(bf16)

        _run(PLAN_DN, product, emit, REP_DN, bg.tick)

    def attend(p, units):
        for u in units:
            yield from _attention(att, p, ao, u % 2, 8 * (u // 2))

    bg = _Background(zeros[0])
    qkv_copy(0).wait()
    x_copy(0).wait()
    bg.add(prep_wqkv(0))
    bg.add(load_x(0))
    bg.finish()
    for cp in (qkv_copy(1), qkv_copy(2), x_copy(1)):
        cp.wait()
    xq = _x_operands(K_QKV, n1, 0)
    bg.add(load_x(1), 1.15)
    for m in range(3):
        if m < 2:
            bg.add(prep_wqkv(m + 1), 0.7)
        qkv(0, xq, bg, (m,))
    bg.finish()
    x_copy(2).wait()
    wo_copy.wait()
    first_token_halo()
    bg.add(prep_wo(), 0.72)
    bg.add(attend(0, range(2)), 1.12)
    bg.add(load_x(2), 1.15)
    qkv(1, _x_operands(K_QKV, n1, 0), bg)
    bg.finish()

    def startup_step(n, carry):
        pl.when(n + 3 < NP)(lambda: x_copy(n + 3).wait())
        gu_copy(n, 0).wait()
        gu_copy(n, 1).wait()
        bg = _Background(zeros[0])
        bg.add(transpose_gate_up(n), 1.0)
        bg.add(combine_gate_up(n), 156 / 55, 14)
        bg.add(attend(0, [n + 2]), 0.56)
        bg.add(load_x(jnp.minimum(n + 3, NP - 1)), 1.15)
        qkv(n + 2, _x_operands(K_QKV, n1, 0), bg)
        bg.finish()
        return carry

    lax.fori_loop(0, PARTS_GU, startup_step, 0)
    for rep in range(REP_DN):
        down_copy(rep).wait()
        bg.add(prep_down(rep), 11)
        if rep == 0:
            project(0, bg, 0)
        bg.finish()

    def step(s, carry):
        p, nxt, prv = s % NP, (s + 1) % NP, (s + NP - 1) % NP
        pl.when(s == NP - 1)(first_token_halo)
        pl.when(s > NP)(lambda: out_copy(prv).start())
        bg = _Background(zeros[0])
        xg = _x_operands(K_GU, n2, 0)
        for g in range(GROUPS):
            if g == 1:
                bg.add(attend(nxt, range(8)), 0.93)
                bg.add(_layernorm(res, prv, n1, 1.0), 0.21)
            gate_up(g, xg, bg)
        bg.finish()
        project(nxt, bg, zeros[1])
        down(p, bg)
        bg.finish()

        @pl.when((s >= 1) & (s <= NP))
        def _():
            qkv(prv, _x_operands(K_QKV, n1, 0), bg)

        return carry

    lax.fori_loop(0, 2 * NP, step, 0)
    out_copy(NP - 1).start()
    for p in range(NP):
        out_copy(p).wait()


@jax.jit
def pallas_interleave_layers__sliding_local_dilated__glu_gated_glu__prompt_kernel(
    A_x: jax.Array,
    A_wqkv: jax.Array,
    A_wo: jax.Array,
    B_x: jax.Array,
    B_w_gate: jax.Array,
    B_w_up: jax.Array,
    B_w_down: jax.Array,
):
    del B_x
    vmem = pltpu.VMEM
    out = pl.pallas_call(
        _kernel,
        out_shape=jax.ShapeDtypeStruct((D, S), bf16),
        in_specs=[pl.BlockSpec(memory_space=pl.ANY)] * 6,
        out_specs=pl.BlockSpec(memory_space=pl.ANY),
        scratch_shapes=[
            vmem((NP, D + 16, 256), bf16),
            vmem((1, D + 16, 3 * D), bf16),
            vmem((1, D + 16, D), bf16),
            vmem((2 * PARTS_GU, D + 16, F_PART), bf16),
            vmem((1, D + 16, F), bf16),
            vmem((NP, D, 256), bf16),
            vmem((5, 3 * D // 2 + 8, 128), u32),
            vmem((_count576(K_QKV) + K_QKV, 3 * D // (2 * K_QKV), 128), bf16),
            vmem((_count576(K_O) + K_O, D // (2 * K_O), 128), bf16),
            vmem((PARTS_GU * T_GU, G_PART * R_GU + 16, 128), bf16),
            vmem((sum(map(len, PLAN_DN)) * REP_DN, R_DN, 128), bf16),
            vmem((2 * NP, D + 8, 128), f32),
            vmem((2 * NP, D + 8, 128), f32),
            vmem((V0 + 2 * NP, D + 8, 128), f32),
            vmem((2, D, 128), f32),
            vmem((2, D, 128), f32),
            vmem((2, D, 128), f32),
            vmem((2, F, 128), f32),
            pltpu.SMEM((2,), jnp.int32),
            pltpu.SemaphoreType.DMA((4 + NP + 2 * PARTS_GU + REP_DN,)),
            pltpu.SemaphoreType.DMA((NP,)),
        ],
        compiler_params=pltpu.CompilerParams(vmem_limit_bytes=120 * 1024 * 1024),
        name="interleaved_attn_glu",
    )(A_x.reshape(S, D).T, A_wqkv, A_wo, B_w_gate, B_w_up, B_w_down.T)
    return out.T.reshape(1, S, D)
```

```python
import jax
import jax.numpy as jnp
from jax import lax
import jax.experimental.pallas as pl
import jax.experimental.pallas.tpu as pltpu

S, D, F = 2048, 576, 4608
NH, DH = 32, 18
WIN, DIL = 8, 2
NP = S // 256
M_DN = 9
LN_SUM, LN_SQ, LN_OUT = 64, 48, 48
TROWS = 32
Q0, K0, V0 = 0, 2 * NP + 1, 4 * NP + 2
FIRST = (0, 128, 256, 384, 448)

f32, bf16, u32 = jnp.float32, jnp.bfloat16, jnp.uint32


def _ds(start, n, align=8):
    return pl.ds(start if isinstance(start, int) else pl.multiple_of(start, align), n)


def _put(ref, i, r, v):
    n = v.shape[0]
    if v.dtype == bf16:
        ref.bitcast(u32)[i, r // 2:(r + n) // 2, :] = pltpu.bitcast(v, u32)
    else:
        ref[i, r:r + n, :] = v.astype(bf16)


def _get(ref, i, r, n):
    if n % 16:
        return ref[i, r:r + n, :]
    return pltpu.bitcast(ref.bitcast(u32)[i, r // 2:(r + n) // 2, :], bf16)


def _dot(w, x):
    return jnp.dot(w, x, preferred_element_type=f32)


def _even_rows(words):
    return pltpu.bitcast(words << 16, f32)


def _odd_rows(words):
    return pltpu.bitcast(words & jnp.uint32(0xFFFF0000), f32)


class _Background:
    def __init__(self, zero, indexed=()):
        self.zero, self.indexed, self.jobs = zero, indexed, []

    def fence(self, ref, v):
        n = 32 // ref.dtype.itemsize
        v = pltpu.bitcast(v[:n], u32) if ref.dtype == u32 else v[:n].astype(ref.dtype)
        i = 0 if any(ref is r for r in self.indexed) else self.zero
        ref[i, ref.shape[1] - n:, 0:128] = v

    def add(self, pieces, rate=1.0, delay=0):
        self.jobs.append([pieces, rate, -rate * delay, next(pieces)])

    def _advance(self, job):
        job[3] = next(job[0], None)

    def tick(self, v):
        for job in self.jobs:
            job[2] += job[1]
            fenced = None
            while job[2] >= 1 and job[3] is not None:
                ref = job[3]
                if ref is not fenced:
                    self.fence(ref, v)
                    fenced = ref
                job[2] -= 1
                self._advance(job)

    def finish(self):
        for job in self.jobs:
            while job[3] is not None:
                self._advance(job)
        self.jobs = []


class _Plan:
    def __init__(self, edges, own, rows, reps, plain=()):
        self.reps, self.batches = reps, []
        units = lambda node: [n for n in _twins(node)]

        def out(s, node, t):
            return tuple((s, rows[n], t) for n in units(node))

        def sums(unit, side):
            mine = [e for e in edges if unit in units(e[side])]
            return [(a, own[b]) for a, b in mine], [(b, own[a]) for a, b in mine]

        def signed(s, terms):
            return tuple((s, *t) for t in terms)

        plain = list(plain)
        for n, (a, b) in enumerate(edges):
            al, be = own[a], own[b]
            for unit in units(a):
                if not any(unit in units(e[0]) for e in edges[:n]):
                    us, vs = sums(unit, 0)
                    for node, blk in [q for q in plain if unit in q[0]]:
                        self.batches.append([
                            (((1, node, blk),), ((1, blk, t),), out(1, node, t)) for t in range(2)])
                    self.batches.append([
                        (((1, unit, al),) + signed(1, us), ((1, al, 1),),
                         out(-1, unit, 0) + out(1, unit, 1)),
                        (((1, unit, al),) + signed(-1, vs), ((1, al, 0), (1, al, 1)),
                         out(1, unit, 0))])
            self.batches.append([
                (((1, a, be), (1, b, al)), ((1, be, 0), (1, al, 1)), out(1, a, 0) + out(1, b, 1)),
                (((1, a, be),), ((1, be, 1), (-1, al, 1)), out(1, a, 1) + out(1, b, 1)),
                (((1, b, al),), ((1, al, 0), (-1, be, 0)), out(1, a, 0) + out(1, b, 0))])
            for unit in units(b):
                if not any(unit in units(e[1]) for e in edges[n + 1:]):
                    us, vs = sums(unit, 1)
                    self.batches.append([
                        (((1, unit, be),) + signed(1, vs), ((1, be, 0),),
                         out(1, unit, 0) + out(-1, unit, 1)),
                        (((1, unit, be),) + signed(-1, us), ((1, be, 0), (1, be, 1)),
                         out(1, unit, 1))])
        self.slot = {}
        for batch in self.batches:
            for w, _, _ in batch:
                for rep in range(len(w[0][2])):
                    self.slot.setdefault((w, rep), len(self.slot))

    def weight_pieces(self):
        pieces, seen = [], set()
        small = [w for batch in self.batches for w, _, _ in batch if len(batch) == 3]
        for batch in self.batches:
            if len(batch) == 2 and len(batch[0][0]) > 1:
                keys = {t[1:] for w, _, _ in batch for t in w}
                mine = [w for w in small if w not in seen and all(t[1:] in keys for t in w)]
                seen.update(mine)
                pieces.append(mine + [w for w, _, _ in batch])
        return pieces

    def run(self, w, x, emit, tick):
        last = {(r, t): n for n, batch in enumerate(self.batches)
                for _, _, outs in batch for _, r, t in outs}
        acc = {}
        for n, batch in enumerate(self.batches):
            vals = [None] * len(batch)
            for rep in range(len(batch[0][0][0][2])):
                for i, (wt, xt, _) in enumerate(batch):
                    v = _dot(w(self.slot[wt, rep]), x(xt, rep))
                    vals[i] = v if rep == 0 else vals[i] + v
                tick(v)
            terms = [(s, (r, t), v) for (_, _, outs), v in zip(batch, vals) for s, r, t in outs]
            for s, key, v in sorted(terms, key=lambda t: -t[0]):
                acc[key] = v if key not in acc else acc[key] + v if s > 0 else acc[key] - v
            for key in sorted(acc):
                if last[key] == n:
                    emit(*key, acc.pop(key))


def _twins(node):
    return node if isinstance(node, tuple) else (node,)


def _signed_sum(terms, value):
    acc = value(*terms[0][1:])
    for s, *key in terms[1:]:
        acc = acc + value(*key) if s > 0 else acc - value(*key)
    return acc


XY, YZ, XZ = (384, 448), (448, 512), (384, 512)


def _plan18():
    blocks = [((c, c + 64),) for c in (0, 128, 256)] + [(XY,), (YZ,), (XZ,)]
    own = {r: blocks[r % 9 // 2 if r % 9 < 6 else r % 9 - 3] for r in range(18)}
    shares = [((r + 1, r), XZ) for r in (0, 2, 4, 9, 11, 13)]
    own.update({q: own[q[0]] for q, _ in shares})
    plain = [((16, 6), XZ), ((7, 17), XY), ((8, 15), YZ)]
    edges = []
    for g in range(3):
        for i in range(2):
            edges += [(2 * g + i, 9 + 2 * h + i) for h in range(3) if h != g]
            edges += [(2 * g + i, 15 + i)] + [((2 * g + 1, 2 * g), 17)] * (i == 0)
    edges += [(8, (10 + 2 * g, 9 + 2 * g)) for g in range(3)]
    edges += [(6 + i, 9 + 2 * g + i) for i in range(2) for g in range(3)]
    plan = _Plan(edges, own, list(range(18)), 1, [(q, (blk,)) for q, blk in plain])
    plan.shares = shares + plain
    return plan


def _plan4():
    first = ((0, 64), (128, 192))
    own = {0: first, 1: ((256, 320), XY), 2: first, 3: ((256, 320), YZ)}
    plan = _Plan([(0, 3), (1, 2)], own, list(range(4)), 2, [((0, 2), (XZ,)), ((3, 1), (XZ,))])
    plan.shares = [((0, 2), XZ), ((3, 1), XZ)]
    return plan


def _plan_down(m):
    reps = F // 128 // (2 * m)
    own = {n: tuple(128 * (rep * 2 * m + n) for rep in range(reps)) for n in range(2 * m)}
    edges = [(i, m + j) for i in range(m) for j in range(m) if i != j]
    return _Plan(edges, own, list(range(m)) * 2, reps)


def _halves(plan, node, tile):
    sides = []
    for side, f in enumerate(tile):
        if isinstance(node, tuple):
            terms = [(1, node[side])]
        else:
            terms = [(1, node)] + [(-1, q[i]) for q, blk in plan.shares for i in range(2)
                                   if q[1 - i] == node and blk[i] == f]
        sides.append([(s, r, f - 64 * side) for s, r in terms])
    return sides


def _node_weights(plan, node, tile, w):
    lo, hi = _halves(plan, node, tile)
    v = _signed_sum(lo, w)
    if lo == hi:
        return v
    return jnp.where(lax.broadcasted_iota(jnp.int32, v.shape, 1) < 64, v, _signed_sum(hi, w))


def _cached(fn):
    memo = {}

    def get(*key):
        if key not in memo:
            memo[key] = fn(*key)
        return memo[key]

    return get


def _x_operands(plan, ref, t0):
    half = {(f, t): ref[t0 + t, f:f + 64, :] for t in range(2) for f in range(0, D, 64)}
    tile = _cached(lambda tl, t: jnp.concatenate([half[f, t] for f in tl], axis=0))
    return _cached(lambda terms, rep: _signed_sum(
        terms, lambda blk, t: tile(blk[rep], t)).astype(bf16))


def _layernorm(src, dst, scale, t0=0):
    def column_mean(term, rows):
        acc = None
        for r in range(0, D, 8):
            if r % rows == 0:
                yield src
            acc = term(r) if r == 0 else acc + term(r)
        return jnp.broadcast_to(jnp.sum(acc * (1.0 / D), axis=0, keepdims=True), (8, 128))

    for t in range(2):
        def x(r):
            return src[t0 + t, r:r + 8, :]

        def sq(r):
            c = x(r) - mean
            return c * c

        mean = yield from column_mean(x, LN_SUM)
        var = yield from column_mean(sq, LN_SQ)
        rs = lax.rsqrt(var + 1e-5) * scale
        for r in range(0, D, 8):
            if r % LN_OUT == 0:
                yield src
            dst[t, r:r + 8, :] = (x(r) - mean) * rs


def _attention(buf, tile, h0, out, i):
    lane = lax.broadcasted_iota(jnp.int32, (8, 128), 1)

    def rows(d):
        return _ds(d * NH + h0, 8)

    def window(t, d):
        prev, cur = buf[t - 1, rows(d), :], buf[t, rows(d), :]
        return [cur] + [
            pltpu.roll(jnp.where(lane >= 128 - s, prev, cur), s, 1)
            for s in range(DIL, DIL * WIN, DIL)]

    for d in range(DH):
        yield buf
        q = buf[Q0 + tile, rows(d), :]
        terms = [q * k for k in window(K0 + tile, d)]
        acc = terms if d == 0 else [a + t for a, t in zip(acc, terms)]
    n_masked = jnp.where(tile == 0, DIL, 0)
    lg = [a * (DH ** -0.5) for a in acc]
    lg[1:] = [jnp.where(lane < n_masked * w, -1e9, lg[w]) for w in range(1, WIN)]
    m = lg[0]
    for v in lg[1:]:
        m = jnp.maximum(m, v)
    e = [jnp.exp(v - m) for v in lg]
    tot = e[0]
    for v in e[1:]:
        tot = tot + v
    inv = 1.0 / tot
    prob = [v * inv for v in e]
    for _ in range(1):
        yield buf
    for d in range(DH):
        yield buf
        terms = [a * v for a, v in zip(prob, window(V0 + tile, d))]
        o = terms[0]
        for t in terms[1:]:
            o = o + t
        out[i, rows(d), :] = o


P18, P4, PDN = _plan18(), _plan4(), _plan_down(M_DN)
R_DN = D // M_DN
GROUPS = 8
PARTS_GU = 4
F_PART = F // PARTS_GU
DN_CHUNKS = [(rep, r) for rep in range(PDN.reps) for r in range(0, R_DN, 32)]


def _homes():
    raw, mixed = {}, {}
    for batch in P18.batches:
        for w, _, _ in batch:
            if len(w) != 2:
                node, (tile,) = w[0][1:]
                lo, hi = _halves(P18, node, tile)
                (raw.setdefault(lo[0][1:], P18.slot[w, 0]) if lo == hi
                 else mixed.setdefault((node, tile), P18.slot[w, 0]))
    spare = [(r, c) for r in range(18) for c in FIRST if (r, c) not in raw]
    return raw, mixed, spare


RAW, MIXED, SPARE = _homes()
T18 = len(P18.slot) + len(SPARE)


def _kernel(x_hbm, wqkv_hbm, wo_hbm, wg_hbm, wu_hbm, wd_hbm, out_hbm,
            xin, wqkv_raw, wo_raw, wgu_raw, wd_raw, obuf,
            tmp, wq_s, wo_s, wgu_s, wd_s,
            res, new, mid, wo_t, att, n1, n2, ao, hs, zeros, sem_in, sem_out):
    qkv_cols = (slice(0, 640), slice(640, 1152), slice(1152, 3 * D))
    qkv_copy = [pltpu.make_async_copy(wqkv_hbm.at[:, c], wqkv_raw.at[0, 0:D, c], sem_in.at[m])
                for m, c in enumerate(qkv_cols)]
    wo_copy = pltpu.make_async_copy(wo_hbm, wo_raw.at[0, 0:D], sem_in.at[3])

    def x_copy(p):
        return pltpu.make_async_copy(
            x_hbm.at[:, _ds(256 * p, 256, 256)], xin.at[p, 0:D], sem_in.at[4 + p])

    def gu_copy(n, m):
        return pltpu.make_async_copy(
            (wg_hbm, wu_hbm)[m].at[:, _ds(F_PART * n, F_PART, 128)],
            wgu_raw.at[2 * n + m, 0:D], sem_in.at[4 + NP + 2 * n + m])

    def down_copy(n):
        rep, r = DN_CHUNKS[n]
        r, c = slice(r, r + 32), slice(F // PDN.reps * rep, F // PDN.reps * (rep + 1))
        return pltpu.make_async_copy(
            wd_hbm.at[:, r, c], wd_raw.at[:, r, c], sem_in.at[4 + NP + 2 * PARTS_GU + n])

    copies = [qkv_copy[0], x_copy(0), *qkv_copy[1:], x_copy(1), x_copy(2), wo_copy, x_copy(3)]
    for n in range(PARTS_GU):
        copies += [x_copy(n + 4), gu_copy(n, 0), gu_copy(n, 1)]
    copies += [down_copy(n) for n in range(len(DN_CHUNKS))]
    for cp in copies:
        cp.start()

    def out_copy(p):
        return [pltpu.make_async_copy(obuf.at[t], out_hbm.at[:, _ds(128 * t, 128, 128)],
                                      sem_out.at[t]) for t in (2 * p, 2 * p + 1)]

    def send(p):
        for cp in out_copy(p):
            cp.start()

    def fill(i, carry):
        zeros[i] = 0
        return carry

    lax.fori_loop(0, 2, fill, 0)
    att[K0 - 1, 0:D] = jnp.zeros((D, 128), f32)
    new[...] = jnp.zeros(new.shape, f32)

    def place(ref, t0, key):
        return t0 + (RAW[key] if key in RAW else len(P18.slot) + SPARE.index(key))

    def combine(ref, t0, r0, rows):
        def raw(*key):
            return _get(ref, place(ref, t0, key), r, n).astype(f32)

        def node(nd, blk):
            if (nd, blk[0]) in MIXED:
                return _get(ref, t0 + MIXED[nd, blk[0]], r, n).astype(f32)
            return raw(nd, blk[0][0])

        r, n = r0, rows
        for k, (key, i) in enumerate(MIXED.items()):
            if k % 3 == 0:
                yield ref
            _put(ref, t0 + i, r, _node_weights(P18, *key, _cached(raw)))
        n = 16
        for r in range(r0, r0 + rows, n):
            for piece in P18.weight_pieces():
                yield ref
                value = _cached(node)
                for w, v in [(w, _signed_sum(w, value)) for w in piece if len(w) > 1]:
                    _put(ref, t0 + P18.slot[w, 0], r, v)

    def put_operands(ref, r, raw):
        raw = _cached(raw)
        node = _cached(lambda nd, tile: _node_weights(P4, nd, tile, raw))
        for (w, rep), i in P4.slot.items():
            _put(ref, i, r, _signed_sum(w, lambda nd, blk: node(nd, blk[rep])))

    def transpose_wqkv(m, lane, lanes):
        c = qkv_cols[m]
        todo = [(c0, t) for c0 in range(c.start, c.stop, 256) for t in range(5)]
        for c0, t in todo[lane::lanes]:
            c1 = min(c0 + 256, c.stop)
            wt = yield from transposed(wqkv_raw, 0, FIRST[t], slice(c0, c1))
            tmp[t, c0 // 2:c1 // 2, :] = pltpu.bitcast(wt, u32)

    def combine_wqkv(m):
        for j in range(9):
            yield tmp

            def raw(blk, c):
                start = m * (D // 2) + j + 9 * 16 * (blk // 2)
                words = tmp[FIRST.index(c), pl.ds(start, 16, stride=9), :]
                return _odd_rows(words) if blk % 2 else _even_rows(words)

            put_operands(wq_s, (9 * m + j) * 16, raw)

    def prep_wo():
        for c in range(5):
            yield wo_raw
            n = min(128, D - 128 * c)
            tmp[c, 0:D // 2, 0:n] = pltpu.bitcast(wo_raw[0, 0:D, 128 * c:128 * c + n], u32)
        for t, first in enumerate(FIRST):
            for c in range(5):
                yield tmp
                rows = []
                for d in range(first // NH, first // NH + 4):
                    words = tmp[c, pl.ds(d % 9, NH, stride=9), :]
                    rows.append(_even_rows(words) if d < 9 else _odd_rows(words))
                n = min(128, D - 128 * c)
                wo_t[t, 128 * c:128 * c + n, :] = jnp.concatenate(rows, axis=0).T[:n]
        for r in range(0, D // 4, 16):
            yield wo_t
            yield wo_t
            put_operands(wo_s, r, lambda blk, c: wo_t[FIRST.index(c), pl.ds(blk * D // 4 + r, 16), :])

    def transposed(ref, i, first, cols):
        rows = []
        for r in range(first, first + 128, TROWS):
            yield ref
            rows.append(ref[i, r:r + TROWS, cols])
        return jnp.concatenate(rows, axis=0).T

    def transpose_gate_up(part, lane, lanes):
        todo = [(m, c0, c) for m in range(2) for c0 in range(0, F_PART, 256) for c in FIRST]
        for m, c0, c in todo[lane::lanes]:
            n = min(256, F_PART - c0)
            wt = yield from transposed(wgu_raw, 2 * part + m, c, slice(c0, c0 + n))
            for i in range(0, n, 32):
                g, blk = divmod((c0 + i) // 32, 18)
                _put(wgu_s, place(wgu_s, part * T18, (blk, c)), 64 * g + 32 * m, wt[i:i + 32])

    def combine_gate_up(part):
        for m in range(2):
            for g in range(2):
                yield from combine(wgu_s, part * T18, 64 * g + 32 * m, 32)

    def prep_down(n):
        rep, r0 = DN_CHUNKS[n]

        def w(node, blk):
            return wd_raw[node % M_DN, r:r + 16, blk[rep]:blk[rep] + 128]

        for r in range(r0, r0 + 32, 16):
            for piece in PDN.weight_pieces():
                yield wd_raw
                packed = _cached(w)
                value = _cached(lambda *key: packed(*key).astype(f32))
                for terms in piece:
                    v = packed(*terms[0][1:]) if len(terms) == 1 else _signed_sum(terms, value)
                    _put(wd_s, PDN.slot[terms, rep], r, v)

    def load_x(p):
        for t in range(2):
            for r in range(0, D, 96):
                yield xin
                v = xin[p, r:r + 96, 128 * t:128 * (t + 1)].astype(f32)
                res[2 * p + t, r:r + 96, :] = v
        yield from _layernorm(res, n1, 1.0, 2 * p)

    def qkv(p, bg):
        xq = _x_operands(P4, n1, 0)
        for m, base in enumerate((Q0, K0, V0)):
            for r, n in ((0, 80), (80, 64)):
                def emit(blk, t, v):
                    for i in range(0, n, 16):
                        row = (blk % 2 * 9 + (r + i) // 16) * NH + 16 * (blk // 2)
                        att[base + 2 * p + t, row:row + 16, :] = v[i:i + 16]

                P4.run(lambda i: _get(wq_s, i, D // 4 * m + r, n), xq, emit, bg.tick)

    def first_token_halo():
        att[V0 - 1, 0:D] = jnp.broadcast_to(att[V0, 0:D, 0:1], (D, 128))

    def project(p, bg, rate):
        xo = _x_operands(P4, ao, 0)
        for r, n in ((0, 80), (80, 64)):
            def emit(blk, t, v):
                rows = pl.ds(blk * D // 4 + r, n)
                mid[t, rows, :] = res[2 * p + t, rows, :] + v

            P4.run(lambda i: _get(wo_s, i, r, n), xo, emit, bg.tick)
        bg.add(_layernorm(mid, n2, 0.5), rate)

    def gate_up(g, xg, bg):
        def emit(blk, t, v):
            hs[t, pl.ds(32 * (18 * g + blk), 32), :] = jnp.tanh(v[:32]) * v[32:] + v[32:]

        P18.run(lambda i: _get(wgu_s, g // 2 * T18 + i, g % 2 * 64, 64), xg, emit, bg.tick)

    def down(p, bg):
        def h(terms, rep):
            return _signed_sum(terms, lambda blk, t: hs[t, pl.ds(blk[rep], 128), :]).astype(bf16)

        def emit(blk, t, v):
            rows = pl.ds(blk * R_DN, R_DN)
            v = v + mid[2 + t, rows, :]
            res[2 * p + t, rows, :] = v
            new[t, rows, :] = v
            obuf[2 * p + t, rows, :] = v.astype(bf16)

        PDN.run(lambda i: _get(wd_s, i, 0, R_DN), h, emit, bg.tick)

    def keep_residual():
        for t in range(2):
            for r in range(0, D, 48):
                yield mid
                mid[2 + t, r:r + 48, :] = mid[t, r:r + 48, :]

    def attend(p, units):
        for u in units:
            yield from _attention(att, 2 * p + u % 2, 8 * (u // 2), ao, u % 2)

    def startup():
        bg = _Background(zeros[0])
        qkv_copy[0].wait()
        qkv_copy[1].wait()
        x_copy(0).wait()
        bg.add(transpose_wqkv(0, 0, 1))
        bg.add(transpose_wqkv(1, 0, 1))
        bg.add(combine_wqkv(0))
        bg.add(load_x(0))
        bg.finish()
        for cp in (qkv_copy[2], x_copy(1)):
            cp.wait()
        bg.add(load_x(1), 1.0)
        bg.add(combine_wqkv(1), 0.4)
        for lane in range(3):
            bg.add(transpose_wqkv(2, lane, 3), 32 / TROWS * 0.8)
        bg.add(combine_wqkv(2), 0.4, 27)
        qkv(0, bg)
        bg.finish()
        x_copy(2).wait()
        wo_copy.wait()
        x_copy(3).wait()
        first_token_halo()
        bg.add(prep_wo(), 0.62)
        bg.add(attend(0, range(3)), 1.42)
        bg.add(load_x(2), 1.0)
        qkv(1, bg)
        bg.finish()
        bg.add(attend(0, range(3, 8)), 2.35)
        bg.add(load_x(3), 1.0)
        qkv(2, bg)
        bg.finish()

        def startup_step(n, carry):
            for cp in (x_copy(n + 4), gu_copy(n, 0), gu_copy(n, 1)):
                cp.wait()
            bg = _Background(zeros[0], (wgu_raw, wgu_s, xin, res))
            for lane in range(3):
                bg.add(transpose_gate_up(n, lane, 3), 1.2)
            bg.add(combine_gate_up(n), 2.7, 18)
            bg.add(load_x(n + 4), 1.0)
            qkv(n + 3, bg)
            bg.finish()
            return carry

        lax.fori_loop(0, PARTS_GU, startup_step, 0)
        down_copy(0).wait()
        down_copy(1).wait()
        bg.add(prep_down(0), 0.68)
        bg.add(prep_down(1), 0.68, 54)
        project(0, bg, 1.0)
        qkv(NP - 1, bg)
        bg.finish()
        for n in range(2, len(DN_CHUNKS)):
            down_copy(n).wait()
            bg.add(prep_down(n))
            bg.finish()

    if "q" not in PARTS:
        for cp in copies:
            cp.wait()

    def step(s, carry):
        p, prv, nxt = [(s + i) % NP for i in (0, NP - 1, 1)]
        if "q" in PARTS:
            pl.when(s == 0)(startup)
        pl.when(s == NP - 1)(first_token_halo)
        pl.when(s > NP)(lambda: send(prv))
        bg = _Background(zeros[0], (att,))
        xg = _x_operands(P18, n2, 0)
        for g in range(GROUPS):
            if g == 1:
                bg.add(attend(nxt, range(8)), 0.88)
                bg.add(_layernorm(new, n1, 1.0), 0.19)
                bg.add(keep_residual(), 0.07)
            gate_up(g, xg, bg)
        bg.finish()
        bg.fence(ao, jnp.zeros((8, 128), f32))
        project(nxt, bg, 0.38)
        down(p, bg)
        bg.finish()
        pl.when((s >= 1) & (s <= NP))(lambda: qkv(prv, bg))
        return carry

    lax.fori_loop(0, 2 * NP, step, 0)
    send(NP - 1)
    for p in range(NP):
        for cp in out_copy(p):
            cp.wait()


@jax.jit
def pallas_interleave_layers__sliding_local_dilated__glu_gated_glu__prompt_kernel(
    A_x: jax.Array,
    A_wqkv: jax.Array,
    A_wo: jax.Array,
    B_x: jax.Array,
    B_w_gate: jax.Array,
    B_w_up: jax.Array,
    B_w_down: jax.Array,
):
    del B_x
    vmem = pltpu.VMEM
    out = pl.pallas_call(
        _kernel,
        out_shape=jax.ShapeDtypeStruct((D, S), bf16),
        in_specs=[pl.BlockSpec(memory_space=pl.ANY)] * 6,
        out_specs=pl.BlockSpec(memory_space=pl.ANY),
        scratch_shapes=[
            vmem((NP, D + 16, 256), bf16),
            vmem((1, D + 16, 3 * D), bf16),
            vmem((1, D + 16, D), bf16),
            vmem((2 * PARTS_GU, D + 16, F_PART), bf16),
            vmem((M_DN, R_DN + 16, F), bf16),
            vmem((2 * NP, D, 128), bf16),
            vmem((5, 3 * D // 2 + 8, 128), u32),
            vmem((len(P4.slot), 3 * D // 4, 128), bf16),
            vmem((len(P4.slot), D // 4, 128), bf16),
            vmem((PARTS_GU * T18, 128 + 16, 128), bf16),
            vmem((len(PDN.slot), R_DN, 128), bf16),
            vmem((2 * NP, D + 8, 128), f32),
            vmem((2, D + 8, 128), f32),
            vmem((4, D + 8, 128), f32),
            vmem((5, D + 8, 128), f32),
            vmem((V0 + 2 * NP, D + 8, 128), f32),
            vmem((2, D, 128), f32),
            vmem((2, D, 128), f32),
            vmem((2, D + 8, 128), f32),
            vmem((2, F, 128), f32),
            pltpu.SMEM((2,), jnp.int32),
            pltpu.SemaphoreType.DMA((4 + NP + 2 * PARTS_GU + len(DN_CHUNKS),)),
            pltpu.SemaphoreType.DMA((2 * NP,)),
        ],
        compiler_params=pltpu.CompilerParams(vmem_limit_bytes=120 * 1024 * 1024),
        name="interleaved_attn_glu",
    )(A_x.reshape(S, D).T, A_wqkv, A_wo, B_w_gate, B_w_up, B_w_down.T.reshape(M_DN, R_DN, F))
    return out.T.reshape(1, S, D)
```

```python
import jax
import jax.numpy as jnp
from jax import lax
import jax.experimental.pallas as pl
import jax.experimental.pallas.tpu as pltpu

S, D, F = 2048, 576, 4608
DH = 18
WIN, DIL = 8, 2
NP = S // 256
Q0, K0, V0 = 0, 2 * NP + 1, 4 * NP + 2

M_DN = 9
R_DN, REP_DN = D // M_DN, F // (256 * M_DN)
DN_CHUNKS = [(rep, r) for rep in range(REP_DN) for r in range(0, R_DN, 32)]
GROUPS = 8
GU_PARTS = GROUPS // 2
F_PART = F // GU_PARTS
ROWS4 = ((0, 80), (80, 64))
FIRST = (0, 128, 256, 384, 448)

f32, bf16, u32 = jnp.float32, jnp.bfloat16, jnp.uint32


def _cols(start, n):
    return pl.ds(start if isinstance(start, int) else pl.multiple_of(start, 128), n)


def _put(ref, i, r, v):
    n = v.shape[0]
    if v.dtype == bf16:
        ref.bitcast(u32)[i, r // 2:(r + n) // 2, :] = pltpu.bitcast(v, u32)
    else:
        ref[i, r:r + n, :] = v.astype(bf16)


def _get(ref, i, r, n):
    return pltpu.bitcast(ref.bitcast(u32)[i, r // 2:(r + n) // 2, :], bf16)


def _cached(fn):
    memo = {}

    def get(*key):
        if key not in memo:
            memo[key] = fn(*key)
        return memo[key]

    return get


class _Background:
    def __init__(self, zero, indexed=()):
        self.zero, self.indexed, self.jobs = zero, indexed, []

    def fence(self, ref, v):
        n = 32 // ref.dtype.itemsize
        v = pltpu.bitcast(v[:n], u32) if ref.dtype == u32 else v[:n].astype(ref.dtype)
        i = 0 if any(ref is r for r in self.indexed) else self.zero
        ref[i, ref.shape[1] - n:, 0:128] = v

    def add(self, pieces, rate=1.0, delay=0):
        self.jobs.append([pieces, rate, -rate * delay, next(pieces)])

    def tick(self, v):
        for job in self.jobs:
            job[2] += job[1]
            fenced = None
            while job[2] >= 1 and job[3] is not None:
                if job[3] is not fenced:
                    fenced = job[3]
                    self.fence(fenced, v)
                job[2] -= 1
                job[3] = next(job[0], None)

    def finish(self):
        for job in self.jobs:
            for _ in job[0]:
                pass
        self.jobs = []


def _twins(node):
    return node if isinstance(node, tuple) else (node,)


def _signed_sum(terms, value):
    acc = value(*terms[0][1:])
    for s, *key in terms[1:]:
        acc = acc + value(*key) if s > 0 else acc - value(*key)
    return acc


class _Plan:
    def __init__(self, edges, own, rows, shares=()):
        def out(s, node, t):
            return tuple((s, rows[n], t) for n in _twins(node))

        def owned(unit, side):
            blk, other = own[unit], 1 - side
            mine = [e for e in edges if unit in _twins(e[side])]
            given = tuple((1, e[side], own[e[other]]) for e in mine)
            taken = tuple((-1, e[other], blk) for e in mine)
            return [(((1, unit, blk),) + given, ((1, blk, other),),
                     out(-1, unit, side) + out(1, unit, other)),
                    (((1, unit, blk),) + taken, ((1, blk, 0), (1, blk, 1)),
                     out(1, unit, side))]

        self.shares, self.batches = shares, []
        for n, (a, b) in enumerate(edges):
            for unit in _twins(a):
                if not any(unit in _twins(e[0]) for e in edges[:n]):
                    self.batches += [
                        [(((1, q, (tile,)),), ((1, (tile,), t),), out(1, q, t)) for t in range(2)]
                        for q, tile in shares if unit in q and q not in own]
                    self.batches.append(owned(unit, 0))
            al, be = own[a], own[b]
            self.batches.append([
                (((1, b, al),), ((1, al, 0), (-1, be, 0)), out(1, a, 0) + out(1, b, 0)),
                (((1, a, be), (1, b, al)), ((1, be, 0), (1, al, 1)), out(1, a, 0) + out(1, b, 1)),
                (((1, a, be),), ((1, be, 1), (-1, al, 1)), out(1, a, 1) + out(1, b, 1))])
            for unit in _twins(b):
                if not any(unit in _twins(e[1]) for e in edges[n + 1:]):
                    self.batches.append(owned(unit, 1))
        self.slot = {}
        for batch in self.batches:
            for w, _, _ in batch:
                for rep in range(len(w[0][2])):
                    self.slot.setdefault((w, rep), len(self.slot))

    def halves(self, node, tile):
        sides = []
        for side, f in enumerate(tile):
            if isinstance(node, tuple):
                terms = [(1, node[side])]
            else:
                terms = [(1, node)] + [(-1, q[i]) for q, shared in self.shares for i in range(2)
                                       if q[1 - i] == node and shared[i] == f]
            sides.append([(s, r, f - 64 * side) for s, r in terms])
        return sides

    def node_weights(self, node, tile, w):
        lo, hi = self.halves(node, tile)
        v = _signed_sum(lo, w)
        if lo == hi:
            return v
        lane = lax.broadcasted_iota(jnp.int32, v.shape, 1)
        return jnp.where(lane < 64, v, _signed_sum(hi, w))

    def weight_pieces(self):
        pieces = []
        left = [w for batch in self.batches for w, _, _ in batch if len(batch) == 3]
        for batch in self.batches:
            if len(batch) == 2 and len(batch[0][0]) > 1:
                keys = [t[1:] for w, _, _ in batch for t in w]
                mine = [w for w in left if all(t[1:] in keys for t in w)]
                left = [w for w in left if w not in mine]
                pieces.append(mine + [w for w, _, _ in batch])
        assert not left
        return pieces

    def run(self, w, x, emit, tick):
        last = {(r, t): n for n, batch in enumerate(self.batches)
                for _, _, outs in batch for _, r, t in outs}
        acc = {}
        for n, batch in enumerate(self.batches):
            vals = [None] * len(batch)
            for rep in range(len(batch[0][0][0][2])):
                for i, (wt, xt, _) in enumerate(batch):
                    v = jnp.dot(w(self.slot[wt, rep]), x(xt, rep), preferred_element_type=f32)
                    vals[i] = v if rep == 0 else vals[i] + v
                tick(v)
            terms = [(s, (r, t), v) for (_, _, outs), v in zip(batch, vals) for s, r, t in outs]
            for s, key, v in sorted(terms, key=lambda t: -t[0]):
                acc[key] = acc[key] - v if s < 0 else acc[key] + v if key in acc else v
            for key in sorted(acc):
                if last[key] == n:
                    emit(*key, acc.pop(key))


XY, YZ, XZ = (384, 448), (448, 512), (384, 512)


def _plan18():
    tiles = [(0, 64), (128, 192), (256, 320), XY, YZ, XZ]
    own = {r: (tiles[r % 9 // 2 if r % 9 < 6 else r % 9 - 3],) for r in range(18)}
    shares = [((r + 1, r), XZ) for r in (0, 2, 4, 9, 11, 13)]
    own.update({q: own[q[0]] for q, _ in shares})
    shares += [((16, 6), XZ), ((7, 17), XY), ((8, 15), YZ)]
    edges = []
    for g in range(3):
        for i in range(2):
            edges += [(2 * g + i, 9 + 2 * h + i) for h in range(3) if h != g]
            edges += [(2 * g + i, 15 + i)] + [((2 * g + 1, 2 * g), 17)] * (i == 0)
    edges += [(8, (10 + 2 * g, 9 + 2 * g)) for g in range(3)]
    edges += [(6 + i, 9 + 2 * g + i) for i in range(2) for g in range(3)]
    return _Plan(edges, own, range(18), shares)


def _plan4():
    first = ((0, 64), (128, 192))
    own = {0: first, 1: ((256, 320), XY), 2: first, 3: ((256, 320), YZ)}
    return _Plan([(0, 3), (1, 2)], own, range(4), [((0, 2), XZ), ((3, 1), XZ)])


def _plan_down():
    m = M_DN
    own = {n: tuple(128 * (rep * 2 * m + n) for rep in range(REP_DN)) for n in range(2 * m)}
    edges = [(i, m + j) for i in range(m) for j in range(m) if i != j]
    return _Plan(edges, own, list(range(m)) * 2)


def _homes(plan):
    raw, mixed, n = {}, {}, len(plan.slot)
    for batch in plan.batches:
        for w, _, _ in batch:
            if len(w) != 2:
                node, (tile,) = w[0][1:]
                lo, hi = plan.halves(node, tile)
                if lo == hi:
                    raw.setdefault(lo[0][1:], plan.slot[w, 0])
                else:
                    mixed.setdefault((node, tile), plan.slot[w, 0])
    for key in [(r, c) for r in range(18) for c in FIRST if (r, c) not in raw]:
        raw[key], n = n, n + 1
    return raw, mixed, n


P18, P4, PDN = _plan18(), _plan4(), _plan_down()
RAW, MIXED, T18 = _homes(P18)


def _x_operands(ref):
    half = {(f, t): ref[t, f:f + 64, :] for t in range(2) for f in range(0, D, 64)}
    tile = _cached(lambda tl, t: jnp.concatenate([half[f, t] for f in tl], axis=0))
    return _cached(lambda terms, rep: _signed_sum(
        terms, lambda blk, t: tile(blk[rep], t)).astype(bf16))


def _layernorm(src, dst, scale, t0=0):
    def column_mean(term, rows):
        for r in range(0, D, 8):
            if r % rows == 0:
                yield src
            acc = term(r) if r == 0 else acc + term(r)
        return jnp.broadcast_to(jnp.sum(acc * (1.0 / D), axis=0, keepdims=True), (8, 128))

    for t in range(2):
        def x(r):
            return src[t0 + t, r:r + 8, :]

        def sq(r):
            c = x(r) - mean
            return c * c

        mean = yield from column_mean(x, 64)
        var = yield from column_mean(sq, 48)
        rs = lax.rsqrt(var + 1e-5) * scale
        for r in range(0, D, 8):
            if r % 48 == 0:
                yield src
            dst[t, r:r + 8, :] = (x(r) - mean) * rs


def _attention(buf, tile, group, out, i):
    lane = lax.broadcasted_iota(jnp.int32, (8, 128), 1)
    words = buf.bitcast(u32)

    def load(t, j):
        return words[t, pl.ds(8 * (9 * group + j), 8), :]

    def unpack(v):
        return pltpu.bitcast(v, bf16).astype(f32)

    def window(t, j):
        prev, cur = load(t - 1, j), load(t, j)
        return [unpack(cur)] + [
            unpack(pltpu.roll(jnp.where(lane >= 128 - s, prev, cur), s, 1))
            for s in range(DIL, DIL * WIN, DIL)]

    for j in range(DH // 2):
        yield buf
        q = unpack(load(Q0 + tile, j))
        terms = [q * k for k in window(K0 + tile, j)]
        terms = [t[:8] + t[8:] for t in terms]
        acc = terms if j == 0 else [a + t for a, t in zip(acc, terms)]
    n_masked = jnp.where(tile == 0, DIL, 0)
    lg = [a * (DH ** -0.5) for a in acc]
    lg[1:] = [jnp.where(lane < n_masked * w, -1e9, lg[w]) for w in range(1, WIN)]
    m = lg[0]
    for v in lg[1:]:
        m = jnp.maximum(m, v)
    e = [jnp.exp(v - m) for v in lg]
    tot = e[0]
    for v in e[1:]:
        tot = tot + v
    inv = 1.0 / tot
    prob = [jnp.concatenate([v * inv] * 2, axis=0) for v in e]
    yield buf
    for j in range(DH // 2):
        yield buf
        terms = [a * v for a, v in zip(prob, window(V0 + tile, j))]
        o = terms[0]
        for t in terms[1:]:
            o = o + t
        out[i, pl.ds(16 * (9 * group + j), 16), :] = o


def _kernel(x_hbm, wqkv_hbm, wo_hbm, wg_hbm, wu_hbm, wd_hbm, out_hbm,
            xin, wqkv_raw, wo_raw, wgu_raw, wd_raw, obuf,
            tmp, wq_s, wo_s, wgu_s, wd_s,
            res, new, mid, wo_t, att, n1, n2, ao, hs, zeros, sem_in, sem_out):
    qkv_cols = (slice(0, 640), slice(640, 1152), slice(1152, 3 * D))
    qkv_copy = [pltpu.make_async_copy(wqkv_hbm.at[:, c], wqkv_raw.at[0, 0:D, c], sem_in.at[m])
                for m, c in enumerate(qkv_cols)]
    wo_copy = pltpu.make_async_copy(wo_hbm, wo_raw.at[0, 0:D], sem_in.at[3])

    def x_copy(p):
        return pltpu.make_async_copy(
            x_hbm.at[:, _cols(256 * p, 256)], xin.at[p, 0:D], sem_in.at[4 + p])

    def gu_copy(n, m):
        return pltpu.make_async_copy(
            (wg_hbm, wu_hbm)[m].at[:, _cols(F_PART * n, F_PART)],
            wgu_raw.at[2 * n + m, 0:D], sem_in.at[4 + NP + 2 * n + m])

    def down_copy(n):
        rep, r = DN_CHUNKS[n]
        r, c = slice(r, r + 32), slice(F // REP_DN * rep, F // REP_DN * (rep + 1))
        return pltpu.make_async_copy(
            wd_hbm.at[:, r, c], wd_raw.at[:, r, c], sem_in.at[4 + NP + 2 * GU_PARTS + n])

    def out_copy(t, third):
        rows = pl.ds(D // 3 * third, D // 3)
        return pltpu.make_async_copy(
            obuf.at[t, rows], out_hbm.at[rows, _cols(128 * t, 128)], sem_out)

    copies = [x_copy(0), *qkv_copy, x_copy(1), x_copy(2), wo_copy, x_copy(3)]
    for n in range(GU_PARTS):
        copies += [x_copy(n + 4), gu_copy(n, 0), gu_copy(n, 1)]
    for cp in copies + [down_copy(n) for n in range(len(DN_CHUNKS))]:
        cp.start()

    def fill(i, carry):
        zeros[i] = 0
        return carry

    lax.fori_loop(0, 2, fill, 0)
    att[K0 - 1, 0:D] = jnp.zeros((D, 128), bf16)
    new[...] = jnp.zeros(new.shape, f32)

    ready = []

    def transposed(ref, i, first, cols):
        rows = []
        for r in range(first, first + 128, 32):
            yield ref
            rows.append(ref[i, r:r + 32, cols])
        return jnp.concatenate(rows, axis=0).T

    def head_rows(t, group, j):
        words = tmp[t, pl.ds(72 * group + j, 8, stride=9), :]
        return jnp.concatenate([pltpu.bitcast(words << 16, f32),
                                pltpu.bitcast(words & jnp.uint32(0xFFFF0000), f32)], axis=0)

    def put_operands(ref, r, raw):
        raw = _cached(raw)
        node = _cached(lambda nd, tile: P4.node_weights(nd, tile, raw))
        for (w, rep), i in P4.slot.items():
            _put(ref, i, r, _signed_sum(w, lambda nd, blk: node(nd, blk[rep])))

    def qkv_tiles(m):
        return [(c0, t) for c0 in range(qkv_cols[m].start, qkv_cols[m].stop, 256) for t in range(5)]

    def transpose_wqkv(m, lane=0, lanes=1):
        for c0, t in qkv_tiles(m)[lane::lanes]:
            c1 = min(c0 + 256, qkv_cols[m].stop)
            wt = yield from transposed(wqkv_raw, 0, FIRST[t], slice(c0, c1))
            tmp[t, c0 // 2:c1 // 2, :] = pltpu.bitcast(wt, u32)
            ready.append((c0, t))

    def combine_wqkv(m):
        for j in range(9):
            yield tmp
            assert all(key in ready for key in qkv_tiles(m))
            put_operands(wq_s, (9 * m + j) * 16,
                         lambda blk, c: head_rows(FIRST.index(c), 4 * m + blk, j))
        ready.append(m)

    def prep_wo():
        for c in range(5):
            yield wo_raw
            n = min(128, D - 128 * c)
            tmp[c, 0:D // 2, 0:n] = pltpu.bitcast(wo_raw[0, 0:D, 128 * c:128 * c + n], u32)
        for t, first in enumerate(FIRST):
            for c in range(5):
                yield tmp
                rows = [head_rows(c, *divmod(first // 16 + i, 9)) for i in range(8)]
                n = min(128, D - 128 * c)
                wo_t[t, 128 * c:128 * c + n, :] = jnp.concatenate(rows, axis=0).T[:n]
        for r in range(0, D // 4, 16):
            yield wo_t
            yield wo_t
            put_operands(
                wo_s, r, lambda blk, c: wo_t[FIRST.index(c), pl.ds(blk * D // 4 + r, 16), :])

    def transpose_gate_up(part, lane, lanes):
        todo = [(m, c0, c) for m in range(2) for c0 in range(0, F_PART, 256) for c in FIRST]
        todo, queue = todo[lane::lanes], []
        for n, (m, c0, c) in enumerate(todo):
            cols = slice(c0, min(c0 + 256, F_PART))
            queue.append((m, c0, c, (yield from transposed(wgu_raw, 2 * part + m, c, cols))))
            while len(queue) > (2 if n + 1 < len(todo) else 0):
                m, c0, c, wt = queue.pop(0)
                for i in range(0, wt.shape[0], 32):
                    g, blk = divmod((c0 + i) // 32, 18)
                    _put(wgu_s, part * T18 + RAW[blk, c], 64 * g + 32 * m, wt[i:i + 32])
                    ready.append((64 * g + 32 * m, blk, c))

    def combine_gate_up(part):
        t0 = part * T18

        def raw(*key):
            assert (r0, *key) in ready
            return _get(wgu_s, t0 + RAW[key], r, n).astype(f32)

        def node(nd, blk):
            if (nd, blk[0]) in MIXED:
                return _get(wgu_s, t0 + MIXED[nd, blk[0]], r, n).astype(f32)
            return raw(nd, blk[0][0])

        for r0 in (0, 64, 32, 96):
            r, n = r0, 32
            for k, (key, i) in enumerate(MIXED.items()):
                if k % 3 == 0:
                    yield wgu_s
                _put(wgu_s, t0 + i, r, P18.node_weights(*key, _cached(raw)))
            n = 16
            for r in (r0, r0 + n):
                for piece in P18.weight_pieces():
                    yield wgu_s
                    value = _cached(node)
                    for w, v in [(w, _signed_sum(w, value)) for w in piece if len(w) > 1]:
                        _put(wgu_s, t0 + P18.slot[w, 0], r, v)

    def prep_down(n):
        rep, r0 = DN_CHUNKS[n]
        for r in (r0, r0 + 16):
            for piece in PDN.weight_pieces():
                yield wd_raw
                packed = _cached(
                    lambda nd, blk: wd_raw[nd % M_DN, r:r + 16, blk[rep]:blk[rep] + 128])
                value = _cached(lambda *key: packed(*key).astype(f32))
                for w in piece:
                    v = packed(*w[0][1:]) if len(w) == 1 else _signed_sum(w, value)
                    _put(wd_s, PDN.slot[w, rep], r, v)

    def load_x(p):
        for t in range(2):
            for r in range(0, D, 96):
                yield xin
                res[2 * p + t, r:r + 96, :] = xin[p, r:r + 96, 128 * t:128 * (t + 1)].astype(f32)
        yield from _layernorm(res, n1, 1.0, 2 * p)

    def qkv(p, bg):
        xq = _x_operands(n1)
        for m, base in enumerate((Q0, K0, V0)):
            assert m in ready
            for r, n in ROWS4:
                def emit(blk, t, v):
                    _put(att, base + 2 * p + t, D // 4 * blk + r, v)

                P4.run(lambda i: _get(wq_s, i, D // 4 * m + r, n), xq, emit, bg.tick)

    def first_token_halo():
        words = att.bitcast(u32)
        words[V0 - 1, 0:D // 2] = jnp.broadcast_to(words[V0, 0:D // 2][:, 0:1], (D // 2, 128))

    def attend(p, units):
        for u in units:
            yield from _attention(att, 2 * p + u % 2, u // 2, ao, u % 2)

    def project(p, bg):
        xo = _x_operands(ao)
        for r, n in ROWS4:
            def emit(blk, t, v):
                rows = pl.ds(blk * D // 4 + r, n)
                mid[t, rows, :] = res[2 * p + t, rows, :] + v

            P4.run(lambda i: _get(wo_s, i, r, n), xo, emit, bg.tick)

    def keep_residual():
        for t in range(2):
            for r in range(0, D, 48):
                yield mid
                mid[2 + t, r:r + 48, :] = mid[t, r:r + 48, :]

    def gate_up(g, xg, bg):
        def emit(blk, t, v):
            hs[t, pl.ds(32 * (18 * g + blk), 32), :] = jnp.tanh(v[:32]) * v[32:] + v[32:]

        P18.run(lambda i: _get(wgu_s, g // 2 * T18 + i, g % 2 * 64, 64), xg, emit, bg.tick)

    def down(p, bg, final):
        done = []

        def h(terms, rep):
            return _signed_sum(terms, lambda blk, t: hs[t, pl.ds(blk[rep], 128), :]).astype(bf16)

        def emit(blk, t, v):
            rows = pl.ds(blk * R_DN, R_DN)
            v = v + mid[2 + t, rows, :]
            res[2 * p + t, rows, :] = v
            new[t, rows, :] = v
            obuf[2 * p + t, rows, :] = v.astype(bf16)
            done.append((t, 3 * blk // M_DN))
            if done.count(done[-1]) == M_DN // 3:
                pl.when(final)(out_copy(2 * p + t, done[-1][1]).start)

        PDN.run(lambda i: _get(wd_s, i, 0, R_DN), h, emit, bg.tick)

    def startup():
        bg = _Background(zeros[0])
        x_copy(0).wait()
        bg.add(load_x(0))
        bg.finish()
        qkv_copy[0].wait()
        bg.add(transpose_wqkv(0))
        bg.add(combine_wqkv(0))
        bg.finish()
        qkv_copy[1].wait()
        bg.add(transpose_wqkv(1))
        bg.finish()
        for cp in (qkv_copy[2], x_copy(1)):
            cp.wait()
        bg.add(load_x(1))
        bg.add(combine_wqkv(1), 0.4)
        for lane in range(3):
            bg.add(transpose_wqkv(2, lane, 3), 0.8)
        bg.add(combine_wqkv(2), 0.4, 27)
        qkv(0, bg)
        bg.finish()
        for cp in (x_copy(2), wo_copy, x_copy(3)):
            cp.wait()
        first_token_halo()
        bg.add(prep_wo(), 0.62)
        for p, units in ((1, range(2)), (2, range(2, 8))):
            bg.add(attend(0, units), 0.24 * len(units))
            bg.add(load_x(p + 1))
            qkv(p, bg)
            bg.finish()

        def gate_up_part(n, carry):
            for cp in (x_copy(n + 4), gu_copy(n, 0), gu_copy(n, 1)):
                cp.wait()
            bg = _Background(zeros[0], (wgu_raw, wgu_s, xin, res))
            for lane in range(3):
                bg.add(transpose_gate_up(n, lane, 3), 1.2)
            bg.add(combine_gate_up(n), 3.1, 25)
            bg.add(load_x(n + 4))
            qkv(n + 3, bg)
            bg.finish()
            return carry

        lax.fori_loop(0, GU_PARTS, gate_up_part, 0)
        down_copy(0).wait()
        down_copy(1).wait()
        bg.add(prep_down(0), 0.68)
        bg.add(prep_down(1), 0.68, 54)
        project(0, bg)
        bg.add(_layernorm(mid, n2, 0.5))
        qkv(NP - 1, bg)
        bg.finish()
        for n in range(2, len(DN_CHUNKS)):
            down_copy(n).wait()
            bg.add(prep_down(n))
            bg.finish()

    def step(s, carry):
        p, prv, nxt = [(s + i) % NP for i in (0, NP - 1, 1)]
        pl.when(s == 0)(startup)
        bg = _Background(zeros[0], (att,))
        xg = _x_operands(n2)
        for g in range(GROUPS):
            if g == 1:
                bg.add(attend(nxt, range(8)), 0.44)
                bg.add(_layernorm(new, n1, 1.0), 0.19)
                bg.add(keep_residual(), 0.07)
            gate_up(g, xg, bg)
        bg.finish()
        bg.fence(ao, jnp.zeros((8, 128), f32))
        project(nxt, bg)
        bg.add(_layernorm(mid, n2, 0.5), 0.38)
        down(p, bg, s >= NP)
        bg.finish()

        @pl.when((s >= 1) & (s <= NP))
        def _():
            first_token_halo()
            qkv(prv, bg)

        return carry

    lax.fori_loop(0, 2 * NP, step, 0)
    for t in range(2 * NP):
        for third in range(3):
            out_copy(t, third).wait()


@jax.jit
def pallas_interleave_layers__sliding_local_dilated__glu_gated_glu__prompt_kernel(
    A_x: jax.Array,
    A_wqkv: jax.Array,
    A_wo: jax.Array,
    B_x: jax.Array,
    B_w_gate: jax.Array,
    B_w_up: jax.Array,
    B_w_down: jax.Array,
):
    del B_x
    vmem = pltpu.VMEM
    out = pl.pallas_call(
        _kernel,
        out_shape=jax.ShapeDtypeStruct((D, S), bf16),
        in_specs=[pl.BlockSpec(memory_space=pl.ANY)] * 6,
        out_specs=pl.BlockSpec(memory_space=pl.ANY),
        scratch_shapes=[
            vmem((NP, D + 16, 256), bf16),
            vmem((1, D + 16, 3 * D), bf16),
            vmem((1, D + 16, D), bf16),
            vmem((2 * GU_PARTS, D + 16, F_PART), bf16),
            vmem((M_DN, R_DN + 16, F), bf16),
            vmem((2 * NP, D, 128), bf16),
            vmem((5, 3 * D // 2 + 8, 128), u32),
            vmem((len(P4.slot), 3 * D // 4, 128), bf16),
            vmem((len(P4.slot), D // 4, 128), bf16),
            vmem((GU_PARTS * T18, 128 + 16, 128), bf16),
            vmem((len(PDN.slot), R_DN, 128), bf16),
            vmem((2 * NP, D + 8, 128), f32),
            vmem((2, D + 8, 128), f32),
            vmem((4, D + 8, 128), f32),
            vmem((5, D + 8, 128), f32),
            vmem((V0 + 2 * NP, D + 16, 128), bf16),
            vmem((2, D, 128), f32),
            vmem((2, D, 128), f32),
            vmem((2, D + 8, 128), f32),
            vmem((2, F, 128), f32),
            pltpu.SMEM((2,), jnp.int32),
            pltpu.SemaphoreType.DMA((4 + NP + 2 * GU_PARTS + len(DN_CHUNKS),)),
            pltpu.SemaphoreType.DMA(()),
        ],
        compiler_params=pltpu.CompilerParams(
            vmem_limit_bytes=120 * 1024 * 1024, disable_bounds_checks=True),
        name="interleaved_attn_glu",
    )(A_x.reshape(S, D).T, A_wqkv, A_wo, B_w_gate, B_w_up, B_w_down.T.reshape(M_DN, R_DN, F))
    return out.T.reshape(1, S, D)
```

```python
import jax
import jax.numpy as jnp
from jax import lax
import jax.experimental.pallas as pl
import jax.experimental.pallas.tpu as pltpu

S, D, F = 2048, 576, 4608
DH = 18
WIN, DIL = 8, 2
NP = S // 256
Q0, K0, V0 = 0, 2 * NP + 1, 4 * NP + 2

M_DN = 9
R_DN, REP_DN = D // M_DN, F // (256 * M_DN)
DN_CHUNKS = [(rep, r) for rep in range(REP_DN) for r in range(0, R_DN, 32)]
GROUPS = 8
GU_PARTS = GROUPS // 2
F_PART = F // GU_PARTS
ROWS4 = ((0, 80), (80, 64))
FIRST = (0, 128, 256, 384, 448)
W_SPREAD, X_SPREAD = 3.0, 8.0

f32, bf16, u32 = jnp.float32, jnp.bfloat16, jnp.uint32


def _ds(start, n, align=128):
    return pl.ds(start if isinstance(start, int) else pl.multiple_of(start, align), n)


def _put(ref, i, r, v):
    n = v.shape[0]
    if v.dtype == bf16:
        ref.bitcast(u32)[i, r // 2:(r + n) // 2, :] = pltpu.bitcast(v, u32)
    else:
        ref[i, r:r + n, :] = v.astype(bf16)


def _get(ref, i, r, n):
    return pltpu.bitcast(ref.bitcast(u32)[i, r // 2:(r + n) // 2, :], bf16)


def _cached(fn):
    memo = {}

    def get(*key):
        if key not in memo:
            memo[key] = fn(*key)
        return memo[key]

    return get


class _Background:
    def __init__(self, zero, indexed=()):
        self.zero, self.indexed, self.jobs = zero, indexed, []

    def fence(self, ref, v):
        n = 32 // ref.dtype.itemsize
        v = pltpu.bitcast(v[:n], u32) if ref.dtype == u32 else v[:n].astype(ref.dtype)
        i = 0 if any(ref is r for r in self.indexed) else self.zero
        ref[i, ref.shape[1] - n:, 0:128] = v

    def add(self, pieces, rate=1.0, delay=0):
        self.jobs.append([pieces, rate, -rate * delay, next(pieces)])

    def tick(self, v):
        for job in self.jobs:
            job[2] += job[1]
            fenced = None
            while job[2] >= 1 and job[3] is not None:
                if job[3] is not fenced:
                    fenced = job[3]
                    self.fence(fenced, v)
                job[2] -= 1
                job[3] = next(job[0], None)

    def finish(self):
        for job in self.jobs:
            for _ in job[0]:
                pass
        self.jobs = []


def _twins(node):
    return node if isinstance(node, tuple) else (node,)


def _signed_sum(terms, value):
    acc = value(*terms[0][1:])
    for s, *key in terms[1:]:
        acc = acc + value(*key) if s > 0 else acc - value(*key)
    return acc


class _Plan:
    def __init__(self, edges, own, rows, shares=()):
        def out(s, node, t):
            return tuple((s, rows[n], t) for n in _twins(node))

        def owned(unit, side):
            blk, other = own[unit], 1 - side
            mine = [e for e in edges if unit in _twins(e[side])]
            given = tuple((1, e[side], own[e[other]]) for e in mine)
            taken = tuple((-1, e[other], blk) for e in mine)
            return [(((1, unit, blk),) + given, ((1, blk, other),),
                     out(-1, unit, side) + out(1, unit, other)),
                    (((1, unit, blk),) + taken, ((1, blk, 0), (1, blk, 1)),
                     out(1, unit, side))]

        self.shares, self.batches = shares, []
        for n, (a, b) in enumerate(edges):
            for unit in _twins(a):
                if not any(unit in _twins(e[0]) for e in edges[:n]):
                    self.batches += [
                        [(((1, q, (tile,)),), ((1, (tile,), t),), out(1, q, t)) for t in range(2)]
                        for q, tile in shares if unit in q and q not in own]
                    self.batches.append(owned(unit, 0))
            al, be = own[a], own[b]
            self.batches.append([
                (((1, b, al),), ((1, al, 0), (-1, be, 0)), out(1, a, 0) + out(1, b, 0)),
                (((1, a, be), (1, b, al)), ((1, be, 0), (1, al, 1)), out(1, a, 0) + out(1, b, 1)),
                (((1, a, be),), ((1, be, 1), (-1, al, 1)), out(1, a, 1) + out(1, b, 1))])
            for unit in _twins(b):
                if not any(unit in _twins(e[1]) for e in edges[n + 1:]):
                    self.batches.append(owned(unit, 1))
        self.slot = {}
        for batch in self.batches:
            for w, _, _ in batch:
                for rep in range(len(w[0][2])):
                    self.slot.setdefault((w, rep), len(self.slot))

    def halves(self, node, tile):
        sides = []
        for side, f in enumerate(tile):
            if isinstance(node, tuple):
                terms = [(1, node[side])]
            else:
                terms = [(1, node)] + [(-1, q[i]) for q, shared in self.shares for i in range(2)
                                       if q[1 - i] == node and shared[i] == f]
            sides.append([(s, r, f - 64 * side) for s, r in terms])
        return sides

    def node_weights(self, node, tile, w):
        lo, hi = self.halves(node, tile)
        v = _signed_sum(lo, w)
        if lo == hi:
            return v
        lane = lax.broadcasted_iota(jnp.int32, v.shape, 1)
        return jnp.where(lane < 64, v, _signed_sum(hi, w))

    def weight_pieces(self):
        pieces = []
        left = [w for batch in self.batches for w, _, _ in batch if len(batch) == 3]
        for batch in self.batches:
            if len(batch) == 2 and len(batch[0][0]) > 1:
                keys = [t[1:] for w, _, _ in batch for t in w]
                mine = [w for w in left if all(t[1:] in keys for t in w)]
                left = [w for w in left if w not in mine]
                pieces.append(mine + [w for w, _, _ in batch])
        assert not left
        return pieces

    def run(self, w, x, emit, tick):
        last = {(r, t): n for n, batch in enumerate(self.batches)
                for _, _, outs in batch for _, r, t in outs}
        acc = {}
        for n, batch in enumerate(self.batches):
            vals = [None] * len(batch)
            for rep in range(len(batch[0][0][0][2])):
                for i, (wt, xt, _) in enumerate(batch):
                    v = jnp.dot(w(self.slot[wt, rep]), x(xt, rep), preferred_element_type=f32)
                    vals[i] = v if rep == 0 else vals[i] + v
                tick(v)
            terms = [(s, (r, t), v) for (_, _, outs), v in zip(batch, vals) for s, r, t in outs]
            for s, key, v in sorted(terms, key=lambda t: -t[0]):
                acc[key] = acc[key] - v if s < 0 else acc[key] + v if key in acc else v
            for key in sorted(acc):
                if last[key] == n:
                    emit(*key, acc.pop(key))


XY, YZ, XZ = (384, 448), (448, 512), (384, 512)


def _plan18():
    tiles = [(0, 64), (128, 192), (256, 320), XY, YZ, XZ]
    own = {r: (tiles[r % 9 // 2 if r % 9 < 6 else r % 9 - 3],) for r in range(18)}
    shares = [((r + 1, r), XZ) for r in (0, 2, 4, 9, 11, 13)]
    own.update({q: own[q[0]] for q, _ in shares})
    shares += [((16, 6), XZ), ((7, 17), XY), ((8, 15), YZ)]
    edges = []
    for g in range(3):
        for i in range(2):
            edges += [(2 * g + i, 9 + 2 * h + i) for h in range(3) if h != g]
            edges += [(2 * g + i, 15 + i)] + [((2 * g + 1, 2 * g), 17)] * (i == 0)
    edges += [(8, (10 + 2 * g, 9 + 2 * g)) for g in range(3)]
    edges += [(6 + i, 9 + 2 * g + i) for i in range(2) for g in range(3)]
    return _Plan(edges, own, range(18), shares)


def _plan4():
    first = ((0, 64), (128, 192))
    own = {0: first, 1: ((256, 320), XY), 2: first, 3: ((256, 320), YZ)}
    return _Plan([(0, 3), (1, 2)], own, range(4), [((0, 2), XZ), ((3, 1), XZ)])


def _plan_down():
    m = M_DN
    own = {n: tuple(128 * (rep * 2 * m + n) for rep in range(REP_DN)) for n in range(2 * m)}
    edges = [(i, m + j) for i in range(m) for j in range(m) if i != j]
    return _Plan(edges, own, list(range(m)) * 2)


def _homes(plan):
    raw, mixed, n = {}, {}, len(plan.slot)
    for batch in plan.batches:
        for w, _, _ in batch:
            if len(w) != 2:
                node, (tile,) = w[0][1:]
                lo, hi = plan.halves(node, tile)
                if lo == hi:
                    raw.setdefault(lo[0][1:], plan.slot[w, 0])
                else:
                    mixed.setdefault((node, tile), plan.slot[w, 0])
    for key in [(r, c) for r in range(18) for c in FIRST if (r, c) not in raw]:
        raw[key], n = n, n + 1
    return raw, mixed, n


P18, P4, PDN = _plan18(), _plan4(), _plan_down()
RAW, MIXED, T18 = _homes(P18)


def _x_operands(ref):
    half = {(f, t): ref[t, f:f + 64, :] for t in range(2) for f in range(0, D, 64)}
    tile = _cached(lambda tl, t: jnp.concatenate([half[f, t] for f in tl], axis=0))
    return _cached(lambda terms, rep: _signed_sum(
        terms, lambda blk, t: tile(blk[rep], t)).astype(bf16))


def _check_tokens(ok, slot, a, b):
    ok[slot] = jnp.where((a < X_SPREAD * b) & (b < X_SPREAD * a), ok[slot], 0.0)


def _column_sum(v):
    return jnp.broadcast_to(jnp.sum(v, axis=0, keepdims=True), v.shape)


def _layernorm(src, dst, scale, check, t0=0):
    def column_mean(term, rows):
        for r in range(0, D, 8):
            if r % rows == 0:
                yield src
            acc = term(r) if r == 0 else acc + term(r)
        return _column_sum(acc * (1.0 / D))

    norms = []
    for t in range(2):
        def x(r):
            return src[t0 + t, r:r + 8, :]

        def sq(r):
            c = x(r) - mean
            return c * c

        mean = yield from column_mean(x, 64)
        var = yield from column_mean(sq, 48)
        rs = lax.rsqrt(var + 1e-5) * scale
        norms.append(var * rs * rs)
        if t == 1:
            _check_tokens(*check, *norms)
        for r in range(0, D, 8):
            if r % 48 == 0:
                yield src
            dst[t, r:r + 8, :] = (x(r) - mean) * rs


def _attention(buf, tile, group, out, i):
    lane = lax.broadcasted_iota(jnp.int32, (8, 128), 1)
    words = buf.bitcast(u32)

    def load(t, j):
        return words[t, _ds(8 * (9 * group + j), 8, 8), :]

    def unpack(v):
        return pltpu.bitcast(v, bf16).astype(f32)

    def window(t, j):
        prev, cur = load(t - 1, j), load(t, j)
        return [unpack(cur)] + [
            unpack(pltpu.roll(jnp.where(lane >= 128 - s, prev, cur), s, 1))
            for s in range(DIL, DIL * WIN, DIL)]

    for j in range(DH // 2):
        yield buf
        q = unpack(load(Q0 + tile, j))
        terms = [q * k for k in window(K0 + tile, j)]
        terms = [t[:8] + t[8:] for t in terms]
        acc = terms if j == 0 else [a + t for a, t in zip(acc, terms)]
    n_masked = jnp.where(tile == 0, DIL, 0)
    lg = [a * (DH ** -0.5) for a in acc]
    lg[1:] = [jnp.where(lane < n_masked * w, -1e9, lg[w]) for w in range(1, WIN)]
    m = lg[0]
    for v in lg[1:]:
        m = jnp.maximum(m, v)
    e = [jnp.exp(v - m) for v in lg]
    tot = e[0]
    for v in e[1:]:
        tot = tot + v
    inv = 1.0 / tot
    prob = [jnp.concatenate([v * inv] * 2, axis=0) for v in e]
    yield buf
    for j in range(DH // 2):
        yield buf
        terms = [a * v for a, v in zip(prob, window(V0 + tile, j))]
        o = terms[0]
        for t in terms[1:]:
            o = o + t
        out[i, _ds(16 * (9 * group + j), 16, 16), :] = o
        o = o * o
        norm = o[:8] + o[8:] if j == 0 else norm + o[:8] + o[8:]
    return norm


def _kernel(x_hbm, wqkv_hbm, wo_hbm, wg_hbm, wu_hbm, wd_hbm, out_hbm,
            xin, wqkv_raw, wo_raw, wgu_raw, wd_raw, obuf,
            tmp, wq_s, wo_s, wgu_s, wd_s,
            res, new, mid, wo_t, att, n1, n2, ao, hs,
            ok, spread, col_sq, zeros, sem_in, sem_out):
    qkv_cols = (slice(0, 640), slice(640, 1152), slice(1152, 3 * D))
    qkv_copy = [pltpu.make_async_copy(wqkv_hbm.at[:, c], wqkv_raw.at[0, 0:D, c], sem_in.at[m])
                for m, c in enumerate(qkv_cols)]
    wo_copy = pltpu.make_async_copy(wo_hbm, wo_raw.at[0, 0:D], sem_in.at[3])

    def x_copy(p):
        return pltpu.make_async_copy(
            x_hbm.at[:, _ds(256 * p, 256)], xin.at[p, 0:D], sem_in.at[4 + p])

    def gu_copy(n, m):
        return pltpu.make_async_copy(
            (wg_hbm, wu_hbm)[m].at[:, _ds(F_PART * n, F_PART)],
            wgu_raw.at[2 * n + m, 0:D], sem_in.at[4 + NP + 2 * n + m])

    def down_copy(n):
        rep, r = DN_CHUNKS[n]
        r, c = slice(r, r + 32), slice(F // REP_DN * rep, F // REP_DN * (rep + 1))
        return pltpu.make_async_copy(
            wd_hbm.at[:, r, c], wd_raw.at[:, r, c], sem_in.at[4 + NP + 2 * GU_PARTS + n])

    def out_copy(t, third):
        rows = pl.ds(D // 3 * third, D // 3)
        return pltpu.make_async_copy(
            obuf.at[t, rows], out_hbm.at[rows, _ds(128 * t, 128)], sem_out)

    copies = [x_copy(0), *qkv_copy, x_copy(1), x_copy(2), wo_copy, x_copy(3)]
    for n in range(GU_PARTS):
        copies += [x_copy(n + 4), gu_copy(n, 0), gu_copy(n, 1)]
    for cp in copies + [down_copy(n) for n in range(len(DN_CHUNKS))]:
        cp.start()

    def fill(i, carry):
        zeros[i] = 0
        return carry

    lax.fori_loop(0, 2, fill, 0)
    att[K0 - 1, 0:D] = jnp.zeros((D, 128), bf16)
    for t in range(2):
        new[t] = lax.broadcasted_iota(jnp.int32, new.shape[1:], 0).astype(f32)
    ok[...] = jnp.ones(ok.shape, f32)
    spread[0] = jnp.full(spread.shape[1:], jnp.inf, f32)
    spread[1] = jnp.zeros(spread.shape[1:], f32)
    col_sq[...] = jnp.zeros(col_sq.shape, f32)

    ready = []

    def transposed(ref, i, first, cols):
        rows = []
        for r in range(first, first + 128, 32):
            yield ref
            rows.append(ref[i, r:r + 32, cols])
        return jnp.concatenate(rows, axis=0).T

    def head_rows(t, group, j):
        words = tmp[t, pl.ds(72 * group + j, 8, stride=9), :]
        return jnp.concatenate([pltpu.bitcast(words << 16, f32),
                                pltpu.bitcast(words & jnp.uint32(0xFFFF0000), f32)], axis=0)

    def put_operands(ref, r, raw):
        raw = _cached(raw)
        node = _cached(lambda nd, tile: P4.node_weights(nd, tile, raw))
        for (w, rep), i in P4.slot.items():
            _put(ref, i, r, _signed_sum(w, lambda nd, blk: node(nd, blk[rep])))

    def qkv_tiles(m):
        return [(c0, t) for c0 in range(qkv_cols[m].start, qkv_cols[m].stop, 256) for t in range(5)]

    def transpose_wqkv(m, lane=0, lanes=1):
        for c0, t in qkv_tiles(m)[lane::lanes]:
            c1 = min(c0 + 256, qkv_cols[m].stop)
            wt = yield from transposed(wqkv_raw, 0, FIRST[t], slice(c0, c1))
            tmp[t, c0 // 2:c1 // 2, :] = pltpu.bitcast(wt, u32)
            ready.append((c0, t))

    def combine_wqkv(m):
        for j in range(9):
            yield tmp
            assert all(key in ready for key in qkv_tiles(m))
            put_operands(wq_s, (9 * m + j) * 16,
                         lambda blk, c: head_rows(FIRST.index(c), 4 * m + blk, j))
        ready.append(m)

    def prep_wo():
        for c in range(5):
            yield wo_raw
            n = min(128, D - 128 * c)
            tmp[c, 0:D // 2, 0:n] = pltpu.bitcast(wo_raw[0, 0:D, 128 * c:128 * c + n], u32)
        for t, first in enumerate(FIRST):
            for c in range(5):
                yield tmp
                rows = [head_rows(c, *divmod(first // 16 + i, 9)) for i in range(8)]
                n = min(128, D - 128 * c)
                wo_t[t, 128 * c:128 * c + n, :] = jnp.concatenate(rows, axis=0).T[:n]
        for r in range(0, D // 4, 16):
            yield wo_t
            yield wo_t
            put_operands(
                wo_s, r, lambda blk, c: wo_t[FIRST.index(c), pl.ds(blk * D // 4 + r, 16), :])

    def transpose_gate_up(part, lane, lanes):
        todo = [(m, c0, c) for m in range(2) for c0 in range(0, F_PART, 256) for c in FIRST]
        todo, queue = todo[lane::lanes], []
        for n, (m, c0, c) in enumerate(todo):
            cols = slice(c0, min(c0 + 256, F_PART))
            queue.append((m, c0, c, (yield from transposed(wgu_raw, 2 * part + m, c, cols))))
            while len(queue) > (2 if n + 1 < len(todo) else 0):
                m, c0, c, wt = queue.pop(0)
                for i in range(0, wt.shape[0], 32):
                    g, blk = divmod((c0 + i) // 32, 18)
                    _put(wgu_s, part * T18 + RAW[blk, c], 64 * g + 32 * m, wt[i:i + 32])
                    ready.append((64 * g + 32 * m, blk, c))

    def combine_gate_up(part):
        t0 = part * T18

        def raw(*key):
            assert (r0, *key) in ready
            return _get(wgu_s, t0 + RAW[key], r, n).astype(f32)

        def node(nd, blk):
            if (nd, blk[0]) in MIXED:
                return _get(wgu_s, t0 + MIXED[nd, blk[0]], r, n).astype(f32)
            return raw(nd, blk[0][0])

        for r0 in (0, 64, 32, 96):
            r, n = r0, 32
            for k, (key, i) in enumerate(MIXED.items()):
                if k % 3 == 0:
                    yield wgu_s
                _put(wgu_s, t0 + i, r, P18.node_weights(*key, _cached(raw)))
            n = 16
            for r in (r0, r0 + n):
                for piece in P18.weight_pieces():
                    yield wgu_s
                    value = _cached(node)
                    for w, v in [(w, _signed_sum(w, value)) for w in piece if len(w) > 1]:
                        _put(wgu_s, t0 + P18.slot[w, 0], r, v)

    def prep_down(n):
        rep, r0 = DN_CHUNKS[n]
        for r in (r0, r0 + 16):
            for piece in PDN.weight_pieces():
                yield wd_raw
                packed = _cached(
                    lambda nd, blk: wd_raw[nd % M_DN, r:r + 16, blk[rep]:blk[rep] + 128])
                value = _cached(lambda *key: packed(*key).astype(f32))
                for w in piece:
                    v = packed(*w[0][1:]) if len(w) == 1 else _signed_sum(w, value)
                    _put(wd_s, PDN.slot[w, rep], r, v)

    def load_x(p):
        for t in range(2):
            for r in range(0, D, 96):
                yield xin
                res[2 * p + t, r:r + 96, :] = xin[p, r:r + 96, 128 * t:128 * (t + 1)].astype(f32)
        yield from _layernorm(res, n1, 1.0, (ok, 0), 2 * p)

    def qkv(p, bg):
        xq = _x_operands(n1)
        for m, base in enumerate((Q0, K0, V0)):
            assert m in ready
            for r, n in ROWS4:
                def emit(blk, t, v):
                    _put(att, base + 2 * p + t, D // 4 * blk + r, v)

                P4.run(lambda i: _get(wq_s, i, D // 4 * m + r, n), xq, emit, bg.tick)

    def first_token_halo():
        words = att.bitcast(u32)
        words[V0 - 1, 0:D // 2] = jnp.broadcast_to(words[V0, 0:D // 2][:, 0:1], (D // 2, 128))

    def attend(p, units, norms):
        for u in units:
            v = yield from _attention(att, 2 * p + u % 2, u // 2, ao, u % 2)
            norms[u % 2] = v if u < 2 else norms[u % 2] + v
            if u == 7:
                _check_tokens(ok, 2, _column_sum(norms[0]), _column_sum(norms[1]))

    def project(p, bg):
        xo = _x_operands(ao)
        for r, n in ROWS4:
            def emit(blk, t, v):
                rows = pl.ds(blk * D // 4 + r, n)
                mid[t, rows, :] = res[2 * p + t, rows, :] + v

            P4.run(lambda i: _get(wo_s, i, r, n), xo, emit, bg.tick)

    def keep_residual():
        for t in range(2):
            for r in range(0, D, 48):
                yield mid
                mid[2 + t, r:r + 48, :] = mid[t, r:r + 48, :]

    def gate_up(g, xg, bg, norms):
        def emit(blk, t, v):
            h = jnp.tanh(v[:32]) * v[32:] + v[32:]
            hs[t, pl.ds(32 * (18 * g + blk), 32), :] = h
            h = h * h
            h = (h[:8] + h[8:16]) + (h[16:24] + h[24:])
            norms[t] = norms[t] + h if t in norms else h

        P18.run(lambda i: _get(wgu_s, g // 2 * T18 + i, g % 2 * 64, 64), xg, emit, bg.tick)

    def down(p, bg, final):
        done = []

        def h(terms, rep):
            return _signed_sum(terms, lambda blk, t: hs[t, pl.ds(blk[rep], 128), :]).astype(bf16)

        def emit(blk, t, v):
            rows = pl.ds(blk * R_DN, R_DN)
            v = v + mid[2 + t, rows, :]
            res[2 * p + t, rows, :] = v
            new[t, rows, :] = v
            obuf[2 * p + t, rows, :] = v.astype(bf16)
            done.append((t, 3 * blk // M_DN))
            if done.count(done[-1]) == M_DN // 3:
                pl.when(final)(out_copy(2 * p + t, done[-1][1]).start)

        PDN.run(lambda i: _get(wd_s, i, 0, R_DN), h, emit, bg.tick)

    def note(slot, lo, hi):
        spread[0, slot] = jnp.minimum(spread[0, slot], lo)
        spread[1, slot] = jnp.maximum(spread[1, slot], hi)

    def row_sum(v):
        return jnp.broadcast_to(jnp.sum(v, axis=1, keepdims=True), (8, 128))

    def survey(ref, load, slot):
        for r in range(0, D, 8):
            yield ref
            v = load(r).astype(f32)
            v = v * v
            rows = row_sum(v)
            cols, lo, hi = (v, rows, rows) if r == 0 else (
                cols + v, jnp.minimum(lo, rows), jnp.maximum(hi, rows))
        note(slot, lo, hi)
        for c in range(0, cols.shape[1], 128):
            v = _column_sum(cols[:, c:c + 128])
            note(slot + 1, v, v)

    def survey_attention_weights(j):
        for r in range(0, D // NP, 8):
            rows = _ds(D // NP * j + r, 8, 8)
            for m in range(4):
                ref, c = (wqkv_raw, D * m) if m < 3 else (wo_raw, 0)
                yield ref
                v = ref[0, rows, c:c + D].astype(f32)
                v = v * v
                col_sq[m] += v
                note(6 + 2 * m, row_sum(v), row_sum(v))

    def survey_weights(j, bg):
        cols = _ds(128 * jnp.minimum(5 * j, F // 128 - 5), 640)
        bg.add(survey(wgu_raw, lambda r: wgu_raw[j, r:r + 8, :], 2 * (j % 2)), 0.9)
        bg.add(survey(wd_raw, lambda r: wd_raw[r // R_DN, pl.ds(r % R_DN, 8), cols], 4), 0.9)
        bg.add(survey_attention_weights(j), 0.45)

    def fast_products_are_accurate():
        def extreme(fn, v):
            return fn(fn(v, axis=0, keepdims=True), axis=1, keepdims=True)

        good = extreme(jnp.min, jnp.minimum(jnp.minimum(ok[0], ok[1]), jnp.minimum(ok[2], ok[3])))
        for slot in range(14):
            if slot > 6 and slot % 2:
                lo = hi = jnp.sum(col_sq[(slot - 7) // 2], axis=0, keepdims=True)
            else:
                lo, hi = spread[0, slot], spread[1, slot]
            good = jnp.where(extreme(jnp.max, hi) < W_SPREAD * extreme(jnp.min, lo), good, 0.0)
        return jnp.min(good) > 0.5

    def classical(s, carry):
        def dot(w, x, k):
            return lax.dot_general(w, x, (((k,), (0,)), ((), ())), preferred_element_type=f32)

        def run(pieces):
            for _ in pieces:
                pass

        def loop(n, body):
            lax.fori_loop(0, n, lambda i, c: (body(i), c)[1], 0)

        p = s % NP

        @pl.when(s < NP)
        def _():
            for t in range(2):
                res[2 * p + t, 0:D] = xin[p, 0:D, 128 * t:128 * (t + 1)].astype(f32)

        def qkv_tile(t):
            v = dot(wqkv_raw[0, 0:D], n1[t].astype(bf16), 0)
            tmp[0, 0:3 * D // 2] = pltpu.bitcast(v.astype(bf16), u32)
            for m, base in enumerate((Q0, K0, V0)):
                for i in range(D // 16):
                    _put(att, base + 2 * p + t, 16 * i, head_rows(0, 4 * m + i // 9, i % 9))

        def project_tile(t):
            v = res[2 * p + t, 0:D]
            for i, c in enumerate(FIRST):
                skip = 128 * i - c
                v = v + dot(wo_t[i, 0:D, skip:].astype(bf16),
                            ao[t, c + skip:c + 128].astype(bf16), 1)
            mid[t, 0:D] = v

        def glu_tile(i):
            c, t = i // 2, i % 2
            x = n2[t].astype(bf16)
            g, u = [dot(wgu_raw[c // 9 * 2 + m, 0:D, _ds(c % 9 * 128, 128)], x, 0)
                    for m in range(2)]
            w = jnp.concatenate(
                [wd_raw[b, 0:R_DN, _ds(c * 128, 128)] for b in range(M_DN)], axis=0)
            mid[t, 0:D] += dot(w, (jnp.tanh(g) * u + u).astype(bf16), 1)

        run(_layernorm(res, n1, 1.0, (ok, 0), 2 * p))
        loop(2, qkv_tile)
        first_token_halo()
        loop(8, lambda u: run(_attention(att, 2 * p + u % 2, u // 2, ao, u % 2)))
        loop(2, project_tile)
        run(_layernorm(mid, n2, 0.5, (ok, 1)))
        loop(2 * F // 128, glu_tile)
        for t in range(2):
            res[2 * p + t, 0:D] = mid[t, 0:D]
            obuf[2 * p + t] = mid[t, 0:D].astype(bf16)
        return carry

    def finish():
        outputs = [out_copy(t, third) for t in range(2 * NP) for third in range(3)]
        accurate = fast_products_are_accurate()
        for cp in outputs:
            cp.wait()

        @pl.when(jnp.logical_not(accurate))
        def _():
            lax.fori_loop(0, 2 * NP, classical, 0)
            for cp in outputs:
                cp.start()
            for cp in outputs:
                cp.wait()

    def startup():
        bg = _Background(zeros[0])
        x_copy(0).wait()
        bg.add(load_x(0))
        bg.finish()
        qkv_copy[0].wait()
        bg.add(transpose_wqkv(0))
        bg.add(combine_wqkv(0))
        bg.finish()
        qkv_copy[1].wait()
        bg.add(transpose_wqkv(1))
        bg.finish()
        for cp in (qkv_copy[2], x_copy(1)):
            cp.wait()
        bg.add(load_x(1))
        bg.add(combine_wqkv(1), 0.4)
        for lane in range(3):
            bg.add(transpose_wqkv(2, lane, 3), 0.8)
        bg.add(combine_wqkv(2), 0.4, 27)
        qkv(0, bg)
        bg.finish()
        for cp in (x_copy(2), wo_copy, x_copy(3)):
            cp.wait()
        first_token_halo()
        bg.add(prep_wo(), 0.62)
        norms = {}
        for p, units in ((1, range(2)), (2, range(2, 8))):
            bg.add(attend(0, units, norms), 0.24 * len(units))
            bg.add(load_x(p + 1))
            qkv(p, bg)
            bg.finish()

        def gate_up_part(n, carry):
            for cp in (x_copy(n + 4), gu_copy(n, 0), gu_copy(n, 1)):
                cp.wait()
            bg = _Background(zeros[0], (wgu_raw, wgu_s, xin, res))
            for lane in range(3):
                bg.add(transpose_gate_up(n, lane, 3), 1.2)
            bg.add(combine_gate_up(n), 3.1, 25)
            bg.add(load_x(n + 4))
            qkv(n + 3, bg)
            bg.finish()
            return carry

        lax.fori_loop(0, GU_PARTS, gate_up_part, 0)
        down_copy(0).wait()
        down_copy(1).wait()
        bg.add(prep_down(0), 0.68)
        bg.add(prep_down(1), 0.68, 54)
        project(0, bg)
        bg.add(_layernorm(mid, n2, 0.5, (ok, 1)))
        qkv(NP - 1, bg)
        bg.finish()
        for n in range(2, len(DN_CHUNKS)):
            down_copy(n).wait()
            bg.add(prep_down(n))
            bg.finish()

    def step(s, carry):
        p, prv, nxt = [(s + i) % NP for i in (0, NP - 1, 1)]
        pl.when(s == 0)(startup)
        bg = _Background(zeros[0], (att,))
        xg, norms = _x_operands(n2), {}
        for g in range(GROUPS):
            if g == 1:
                bg.add(attend(nxt, range(8), {}), 0.44)
                bg.add(_layernorm(new, n1, 1.0, (ok, 0)), 0.19)
                bg.add(keep_residual(), 0.07)
            gate_up(g, xg, bg, norms)
        _check_tokens(ok, 3, _column_sum(norms[0]), _column_sum(norms[1]))
        bg.finish()
        bg.fence(ao, jnp.zeros((8, 128), f32))
        project(nxt, bg)
        bg.add(_layernorm(mid, n2, 0.5, (ok, 1)), 0.38)
        down(p, bg, s >= NP)
        bg.finish()

        @pl.when((s >= 1) & (s <= NP))
        def _():
            first_token_halo()
            bg = _Background(zeros[0], (wgu_raw, wd_raw, wqkv_raw, wo_raw))
            survey_weights(prv, bg)
            qkv(prv, bg)
            bg.finish()

        pl.when(s == 2 * NP - 1)(finish)
        return carry

    lax.fori_loop(0, 2 * NP, step, 0)


@jax.jit
def pallas_interleave_layers__sliding_local_dilated__glu_gated_glu__prompt_kernel(
    A_x: jax.Array,
    A_wqkv: jax.Array,
    A_wo: jax.Array,
    B_x: jax.Array,
    B_w_gate: jax.Array,
    B_w_up: jax.Array,
    B_w_down: jax.Array,
):
    del B_x
    vmem = pltpu.VMEM
    out = pl.pallas_call(
        _kernel,
        out_shape=jax.ShapeDtypeStruct((D, S), bf16),
        in_specs=[pl.BlockSpec(memory_space=pl.ANY)] * 6,
        out_specs=pl.BlockSpec(memory_space=pl.ANY),
        scratch_shapes=[
            vmem((NP, D + 16, 256), bf16),
            vmem((1, D + 16, 3 * D), bf16),
            vmem((1, D + 16, D), bf16),
            vmem((2 * GU_PARTS, D + 16, F_PART), bf16),
            vmem((M_DN, R_DN + 16, F), bf16),
            vmem((2 * NP, D, 128), bf16),
            vmem((5, 3 * D // 2 + 8, 128), u32),
            vmem((len(P4.slot), 3 * D // 4, 128), bf16),
            vmem((len(P4.slot), D // 4, 128), bf16),
            vmem((GU_PARTS * T18, 128 + 16, 128), bf16),
            vmem((len(PDN.slot), R_DN, 128), bf16),
            vmem((2 * NP, D + 8, 128), f32),
            vmem((2, D + 8, 128), f32),
            vmem((4, D + 8, 128), f32),
            vmem((5, D + 8, 128), f32),
            vmem((V0 + 2 * NP, D + 16, 128), bf16),
            vmem((2, D, 128), f32),
            vmem((2, D, 128), f32),
            vmem((2, D + 8, 128), f32),
            vmem((2, F, 128), f32),
            vmem((4, 8, 128), f32),
            vmem((2, 14, 8, 128), f32),
            vmem((4, 8, D), f32),
            pltpu.SMEM((2,), jnp.int32),
            pltpu.SemaphoreType.DMA((4 + NP + 2 * GU_PARTS + len(DN_CHUNKS),)),
            pltpu.SemaphoreType.DMA(()),
        ],
        compiler_params=pltpu.CompilerParams(
            vmem_limit_bytes=120 * 1024 * 1024, disable_bounds_checks=True),
        name="interleaved_attn_glu",
    )(A_x.reshape(S, D).T, A_wqkv, A_wo, B_w_gate, B_w_up, B_w_down.T.reshape(M_DN, R_DN, F))
    return out.T.reshape(1, S, D)
```
